```python
import jax
import jax.numpy as jnp

def _softmax(x, axis=-1):
    return jax.nn.softmax(x, axis=axis)

def _gelu(x):
    return jax.nn.gelu(x, approximate=True)

def _silu(x):
    return jax.nn.silu(x)

def _sigmoid(x):
    return jax.nn.sigmoid(x)

def _layernorm(x, axis=-1, eps=1e-05):
    m = jnp.mean(x, axis=axis, keepdims=True)
    v = jnp.var(x, axis=axis, keepdims=True)
    return (x - m) / jnp.sqrt(v + eps)

def _scatter_add(tgt, idx, src, axis=0):
    return tgt.at[idx].add(src)

def _segment_sum(src, seg, n):
    return jax.ops.segment_sum(src, seg, n)

class _Rng:

    def __init__(self, key):
        self._k = key

    def _next(self):
        self._k, sub = jax.random.split(self._k)
        return sub

    def normal(self, shape):
        return jax.random.normal(self._next(), shape, dtype=jnp.bfloat16)

    def randint(self, lo, hi, shape):
        return jax.random.randint(self._next(), shape, lo, hi, dtype=jnp.int32)

    def uniform(self, shape, lo=0.0, hi=1.0):
        return jax.random.uniform(self._next(), shape, jnp.bfloat16, lo, hi)

    def permutation(self, n):
        return jax.random.permutation(self._next(), n)
kernel_name = 'adaLN_cond__compressed_kv_cla__moe_arch_mod__prompt'

def setup_inputs():
    _rng = _Rng(jax.random.key(int.from_bytes(__import__("os").urandom(4), "little")))
    _w = lambda a: (lambda t: t.astype(jnp.bfloat16) if jnp.issubdtype(t.dtype, jnp.floating) else t)(jnp.asarray(a))

    def _A_setup():
        B, H, Sq, Sk, D, M = (1, 32, 2048, 2048, 128, 640)
        Dc = 4 * D
        return {'x': _w((lambda *s: _rng.normal(s) * 0.05)(B, Sq, M)), 'c_kv': _w((lambda *s: _rng.normal(s) * 0.05)(B, Sk, Dc)), 'w_q': _w((lambda *s: _rng.normal(s) * 0.05)(M, H, D) * M ** (-0.5)), 'w_uk': _w((lambda *s: _rng.normal(s) * 0.05)(Dc, H, D) * Dc ** (-0.5)), 'w_uv': _w((lambda *s: _rng.normal(s) * 0.05)(Dc, H, D) * Dc ** (-0.5)), 'w_o': _w((lambda *s: _rng.normal(s) * 0.05)(H, D, M) * (H * D) ** (-0.5))}
    _A_in = _A_setup()

    def _B_setup():
        B, S, D, F, C = (1, 2048, 640, 1728, 8)
        return {'x': _w((lambda *s: _rng.normal(s) * 0.05)(B, S, D)), 'w_r': _w((lambda *s: _rng.normal(s) * 0.05)(D)), 'w_gate': _w((lambda *s: _rng.normal(s) * 0.05)(D, F)), 'w_up': _w((lambda *s: _rng.normal(s) * 0.05)(D, F)), 'w_down': _w((lambda *s: _rng.normal(s) * 0.05)(F, D))}
    _B_in = _B_setup()
    return {'A_x': _A_in['x'], 'A_c_kv': _A_in['c_kv'], 'A_w_q': _A_in['w_q'], 'A_w_uk': _A_in['w_uk'], 'A_w_uv': _A_in['w_uv'], 'A_w_o': _A_in['w_o'], 'B_x': _B_in['x'], 'B_w_r': _B_in['w_r'], 'B_w_gate': _B_in['w_gate'], 'B_w_up': _B_in['w_up'], 'B_w_down': _B_in['w_down'], 'c': _w((lambda *s: _rng.normal(s) * 0.05)(1, 640)), 'w_mod': _w((lambda *s: _rng.normal(s) * 0.05)(640, 6 * 640) * 640 ** (-0.5))}

def reference(A_x, A_c_kv, A_w_q, A_w_uk, A_w_uv, A_w_o, B_x, B_w_r, B_w_gate, B_w_up, B_w_down, c, w_mod):

    def _A_ref(x, c_kv, w_q, w_uk, w_uv, w_o):
        B, Sq, M = (x.shape[0], x.shape[1], x.shape[2])
        Sk = c_kv.shape[1]
        H, D = (w_q.shape[1], w_q.shape[2])
        q = jnp.einsum('bqm,mhd->bhqd', x, w_q)
        k = jnp.einsum('bkc,chd->bhkd', c_kv, w_uk)
        v = jnp.einsum('bkc,chd->bhkd', c_kv, w_uv)
        scores = jnp.einsum('bhqd,bhkd->bhqk', q, k) * D ** (-0.5)
        off = Sk - Sq
        qi = jnp.arange(Sq)[:, None]
        kj = jnp.arange(Sk)[None, :]
        cmask = kj <= qi + off
        scores = jnp.where(cmask[None, None], scores, -1000000000.0)
        p = _softmax(scores, axis=-1)
        ctx = jnp.einsum('bhqk,bhkd->bhqd', p, v)
        return jnp.einsum('bhqd,hdm->bqm', ctx, w_o)

    def _B_ref(x, w_r, w_gate, w_up, w_down):
        B, S, D = x.shape
        C = 8
        r = x @ w_r
        idx = jnp.argsort(-r, axis=-1)[:, :C]
        idx_e = jnp.repeat(idx.reshape(B, C, 1), D, axis=2)
        x_sel = jnp.take_along_axis(x, idx_e, axis=1)
        g = _silu(x_sel @ w_gate)
        u = x_sel @ w_up
        y = g * u @ w_down
        r_sel = _sigmoid(jnp.take_along_axis(r, idx, axis=1))
        y = y * r_sel.reshape(B, C, 1)
        b_off = (jnp.arange(B) * S).reshape(B, 1)
        flat_idx = (idx + b_off).reshape(B * C)
        zero = (x * 0.0).reshape(B * S, D)
        upd = _scatter_add(zero, flat_idx, y.reshape(B * C, D), axis=0)
        return x + upd.reshape(B, S, D)
    x = A_x
    mod = (_silu(c) @ w_mod).reshape(c.shape[0], 6, 1, -1)
    sa, ca, ga, sb, cb, gb = (mod[:, 0].copy(), mod[:, 1].copy(), mod[:, 2].copy(), mod[:, 3].copy(), mod[:, 4].copy(), mod[:, 5].copy())
    h = _layernorm(x, axis=-1) * (1 + ca) + sa
    x = x + ga * _A_ref(h, A_c_kv, A_w_q, A_w_uk, A_w_uv, A_w_o)
    h = _layernorm(x, axis=-1) * (1 + cb) + sb
    x = x + gb * _B_ref(h, B_w_r, B_w_gate, B_w_up, B_w_down)
    return x
```

```python
import math

import jax
import jax.numpy as jnp
from jax import lax
import jax.experimental.pallas as pl
import jax.experimental.pallas.tpu as pltpu

F32 = jnp.float32
BF16 = jnp.bfloat16
U32 = jnp.uint32
I32 = jnp.int32

_NT = (((1,), (1,)), ((), ()))
_EPS = 1e-5
_TOPC = 8
_BQ = 128
_DEPTH = 2
_HG = 8
_RB = 512


def _rnd(v):
    return v.astype(BF16).astype(F32)


def _adaln_ref_rounding(x, shift, scale):
    mean = jnp.mean(x, axis=1, keepdims=True)
    d = x - mean
    var = _rnd(jnp.mean(d * d, axis=1, keepdims=True))
    den = _rnd(jnp.sqrt(_rnd(var + _rnd(jnp.full((1, 1), _EPS, F32)))))
    n = _rnd(_rnd(x - _rnd(mean)) / den)
    return _rnd(_rnd(n * _rnd(1.0 + scale)) + shift)


def _pack(v):
    return pltpu.bitcast(v.astype(BF16), U32)


def _unpack(v):
    return pltpu.bitcast(v, BF16)


def _kernel(x_hbm, ckv_hbm, wq_hbm, wuk_hbm, wuv_hbm, wo_hbm, wr_hbm, wg_hbm,
            wu_hbm, wd_hbm, c_hbm, wmod_hbm, out_hbm,
            x_v, ckv_v, wq_v, wuk_v, wuv_v, wo_v, wr_v, wg_v, wu_v, wd_v, c_v,
            wmod_v, out_v, wq2_v, k_v, v_v, ctx_v, h_v, mod_v, x1_v, h2_v, r_v, sems,
            *, S, M, H, D, Dc):
    ng = H // _HG

    def group_copy(src, dst, base, g):
        return pltpu.make_async_copy(
            src.at[:, pl.ds(g * _HG, _HG), :], dst.at[g], sems.at[base + g])

    whole = [(ckv_hbm, ckv_v), (c_hbm, c_v), (wmod_hbm, wmod_v), (x_hbm, x_v),
             (wo_hbm, wo_v), (wr_hbm, wr_v), (wg_hbm, wg_v), (wu_hbm, wu_v),
             (wd_hbm, wd_v)]
    cps = [pltpu.make_async_copy(a, b, sems.at[3 * ng + i]) for i, (a, b) in enumerate(whole)]
    cps[0].start()
    for g in range(ng):
        group_copy(wuk_hbm, wuk_v, 0, g).start()
        group_copy(wuv_hbm, wuv_v, ng, g).start()
        group_copy(wq_hbm, wq_v, 2 * ng, g).start()
    for cp in cps[1:]:
        cp.start()

    cps[0].wait()

    def kv_body(g, carry):
        for dst, base in ((wuk_v, 0), (wuv_v, ng), (wq_v, 2 * ng)):
            pltpu.make_async_copy(dst.at[g], dst.at[g], sems.at[base + g]).wait()
        for w_v, o_v in ((wuk_v, k_v), (wuv_v, v_v)):
            w = w_v[g].reshape(Dc, _HG * D)
            r = jnp.dot(ckv_v[...], w, preferred_element_type=F32)
            for e in range(_HG):
                o_v[g * _HG + e] = _pack(r[:, e * D:(e + 1) * D])
        w = wq_v[g].reshape(M, _HG * D)
        for e in range(_HG // 2):
            wq2_v[g * (_HG // 2) + e] = pltpu.bitcast(w[:, 2 * e * D:(2 * e + 2) * D], U32)
        return carry

    lax.fori_loop(0, ng, kv_body, 0)

    for cp in cps[1:4]:
        cp.wait()
    cf = c_v[...].astype(F32)
    sc = jnp.broadcast_to(cf * jax.nn.sigmoid(cf), (16, M)).astype(BF16)
    mod = _rnd(jnp.dot(sc, wmod_v[...], preferred_element_type=F32)[0:1, :])
    for i in range(6):
        mod_v[i:i + 1, :] = mod[:, i * M:(i + 1) * M]

    def ln1_body(b, carry):
        r0 = pl.multiple_of(b * 256, 256)
        xb = x_v[pl.ds(r0, 256), :].astype(F32)
        hb = _adaln_ref_rounding(xb, mod_v[0:1, :], mod_v[1:2, :])
        h_v[pl.ds(pl.multiple_of(b * 128, 128), 128), :] = _pack(hb)
        return carry

    lax.fori_loop(0, S // 256, ln1_body, 0)

    qscale = float(D ** -0.5 * math.log2(math.e))
    neg = float(-1e9 * math.log2(math.e))
    row = lax.broadcasted_iota(I32, (_BQ, _BQ), 0)
    col = lax.broadcasted_iota(I32, (_BQ, _BQ), 1)
    nb = S // _BQ
    hb = _BQ // 2

    def attn_body(j, carry):
        w = _unpack(wq2_v[j])
        q2 = (jnp.dot(_unpack(h_v[...]), w, preferred_element_type=F32) * qscale).astype(BF16)

        def qk(e, i):
            n = i * _BQ
            q = q2[n:n + _BQ, e * D:(e + 1) * D]
            k = _unpack(k_v[2 * j + e, 0:(i + 1) * hb, :])
            s = lax.dot_general(q, k, _NT, preferred_element_type=F32)
            sd = jnp.where(col <= row, s[:, n:], neg)
            s = jnp.concatenate([s[:, :n], sd], axis=1) if n else sd
            return s, jnp.max(s, axis=1, keepdims=True)

        def pv(e, i, s, m):
            p = jnp.exp2(s - m)
            l = jnp.sum(p, axis=1, keepdims=True)
            v = _unpack(v_v[2 * j + e, 0:(i + 1) * hb, :])
            o = jnp.dot(p.astype(BF16), v, preferred_element_type=F32)
            ctx_v[2 * j + e, i * hb:(i + 1) * hb, :] = _pack(o * (1.0 / l))

        pend = []
        for e in range(2):
            for i in reversed(range(nb)):
                pend.append((e, i) + qk(e, i))
                if len(pend) > _DEPTH:
                    pv(*pend.pop(0))
        while pend:
            pv(*pend.pop(0))
        return carry

    lax.fori_loop(0, H // 2, attn_body, 0)

    for cp in cps[4:6]:
        cp.wait()
    wr = jnp.broadcast_to(wr_v[...], (16, M))

    def out_body(b, carry):
        r0 = pl.multiple_of(b * _RB, _RB)
        p0 = pl.multiple_of(b * (_RB // 2), _RB // 2)
        ctx = jnp.concatenate(
            [_unpack(ctx_v[h, pl.ds(p0, _RB // 2), :]) for h in range(H)], axis=1)
        att = _rnd(jnp.dot(ctx, wo_v[...], preferred_element_type=F32))
        x1 = _rnd(x_v[pl.ds(r0, _RB), :].astype(F32) + _rnd(mod_v[2:3, :] * att))
        h2 = _adaln_ref_rounding(x1, mod_v[3:4, :], mod_v[4:5, :])
        x1_v[pl.ds(r0, _RB), :] = x1
        h2_v[pl.ds(r0, _RB), :] = h2
        out_v[pl.ds(r0, _RB), :] = (x1 + _rnd(mod_v[5:6, :] * (h2 + h2 * 0.0))).astype(BF16)
        r = lax.dot_general(wr, h2.astype(BF16), _NT, preferred_element_type=F32)
        r_v[b] = r[0:8, :]
        return carry

    lax.fori_loop(0, S // _RB, out_body, 0)

    nr = S // _RB
    r = _rnd(jnp.concatenate([r_v[b, 0:1, :] for b in range(nr)], axis=0))
    tok = lax.broadcasted_iota(I32, r.shape, 0) * _RB + lax.broadcasted_iota(I32, r.shape, 1)
    bits = pltpu.bitcast(jnp.where(r == 0.0, 0.0, r), I32) >> 16
    order = jnp.where(bits < 0, -(bits & 0x7FFF), bits) + 0x8000
    order = jnp.where(r != r, 0, order)
    key = pltpu.bitcast(((order * S) | (S - 1 - tok)) + 0x20000000, F32)
    idx = []
    for _ in range(_TOPC):
        top = jnp.max(jnp.max(key, axis=1, keepdims=True), axis=0, keepdims=True)
        hit = key == top
        idx.append(jnp.max(jnp.where(hit, tok, 0)))
        key = jnp.where(hit, 0.0, key)

    for cp in cps[6:9]:
        cp.wait()
    hs = jnp.concatenate([h2_v[pl.ds(i, 1), :] for i in idx], axis=0)
    xs = jnp.concatenate([x1_v[pl.ds(i, 1), :] for i in idx], axis=0)
    hs16 = jnp.concatenate([hs, hs], axis=0).astype(BF16)
    g = _rnd(jnp.dot(hs16, wg_v[...], preferred_element_type=F32))
    u = _rnd(jnp.dot(hs16, wu_v[...], preferred_element_type=F32))
    a = (_rnd(g * jax.nn.sigmoid(g)) * u).astype(BF16)
    y = _rnd(jnp.dot(a, wd_v[...], preferred_element_type=F32))[0:_TOPC, :]
    rs = _rnd(jnp.sum(hs * wr_v[...].astype(F32), axis=1, keepdims=True))
    y = _rnd(y * _rnd(jax.nn.sigmoid(rs)))
    new = xs + _rnd(mod_v[5:6, :] * _rnd(hs + _rnd(hs * 0.0 + y)))
    sub = lax.broadcasted_iota(I32, (16, M), 0)
    for n, i in enumerate(idx):
        g0 = pl.multiple_of((i // 16) * 16, 16)
        old = out_v[pl.ds(g0, 16), :].astype(F32)
        out_v[pl.ds(g0, 16), :] = jnp.where(sub == i % 16, new[n:n + 1, :], old).astype(BF16)

    ocp = pltpu.make_async_copy(out_v, out_hbm, sems.at[3 * ng + len(cps)])
    ocp.start()
    ocp.wait()


@jax.jit
def pallas_adaLN_cond__compressed_kv_cla__moe_arch_mod__prompt_kernel(
    A_x: jax.Array,
    A_c_kv: jax.Array,
    A_w_q: jax.Array,
    A_w_uk: jax.Array,
    A_w_uv: jax.Array,
    A_w_o: jax.Array,
    B_x: jax.Array,
    B_w_r: jax.Array,
    B_w_gate: jax.Array,
    B_w_up: jax.Array,
    B_w_down: jax.Array,
    c: jax.Array,
    w_mod: jax.Array,
):
    del B_x
    B, S, M = A_x.shape
    Dc = A_c_kv.shape[2]
    _, H, D = A_w_q.shape
    assert B == 1 and A_c_kv.shape[1] == S

    args = (
        A_x.reshape(S, M), A_c_kv.reshape(S, Dc), A_w_q, A_w_uk, A_w_uv,
        A_w_o.reshape(H * D, M), B_w_r.reshape(1, M), B_w_gate, B_w_up, B_w_down,
        c, w_mod,
    )
    ng = H // _HG
    scratch = [
        pltpu.VMEM((ng, a.shape[0], _HG, D) if a.ndim == 3 else a.shape, a.dtype)
        for a in args
    ] + [
        pltpu.VMEM((S, M), BF16),
        pltpu.VMEM((H // 2, M // 2, 2 * D), U32),
        pltpu.VMEM((H, S // 2, D), U32),
        pltpu.VMEM((H, S // 2, D), U32),
        pltpu.VMEM((H, S // 2, D), U32),
        pltpu.VMEM((S // 2, M), U32),
        pltpu.VMEM((8, M), F32),
        pltpu.VMEM((S, M), F32),
        pltpu.VMEM((S, M), F32),
        pltpu.VMEM((S // _RB, 8, _RB), F32),
        pltpu.SemaphoreType.DMA((3 * ng + len(args) - 2,)),
    ]

    def kernel_function(*refs):
        _kernel(*refs, S=S, M=M, H=H, D=D, Dc=Dc)

    out = pl.pallas_call(
        kernel_function,
        in_specs=[pl.BlockSpec(memory_space=pl.ANY)] * len(args),
        out_specs=pl.BlockSpec(memory_space=pl.ANY),
        out_shape=jax.ShapeDtypeStruct((S, M), A_x.dtype),
        scratch_shapes=scratch,
        compiler_params=pltpu.CompilerParams(vmem_limit_bytes=120 * 1024 * 1024),
        name="adaln_cla_mod",
    )(*args)
    return out.reshape(B, S, M)
```

```python
import functools
import math

import jax
import jax.numpy as jnp
from jax import lax
import jax.experimental.pallas as pl
import jax.experimental.pallas.tpu as pltpu

F32 = jnp.float32
BF16 = jnp.bfloat16
U32 = jnp.uint32
I32 = jnp.int32

_NT = (((1,), (1,)), ((), ()))
_EPS = 1e-5
_TOPC = 8
_BQ = 128
_QC = 256
_HG = 8
_KVR = 256
_LNR = 32
_OR = 128
_FQ = 256
_SUM_EXP = 64
_ACC_EXP = 90
_CKV_ROWS = (256, 256, 512, 1024)
_OUT_ROWS = (512, 512, 512, 256, 128, 128)


def _rnd(v):
    return v.astype(BF16).astype(F32)


def _adaln(x, shift, scale):
    mean = jnp.mean(x, axis=1, keepdims=True)
    d = x - mean
    var = _rnd(jnp.mean(d * d, axis=1, keepdims=True))
    den = _rnd(jnp.sqrt(_rnd(var + _rnd(jnp.full((1, 1), _EPS, F32)))))
    n = _rnd(_rnd(x - _rnd(mean)) / den)
    return _rnd(_rnd(n * _rnd(1.0 + scale)) + shift)


def _pack(v):
    return pltpu.bitcast(v.astype(BF16), U32)


def _unpack(v):
    return pltpu.bitcast(v, BF16)


def _after(words, anchor):
    zero = jnp.where(anchor * anchor < 0.0, jnp.uint32(1), jnp.uint32(0))
    return words | jnp.tile(zero, (words.shape[0] // 8, words.shape[1] // 128))


def _spans(sizes):
    out, start = [], 0
    for n in sizes:
        out.append((start, n))
        start += n
    return out


def _kernel(x_hbm, ckv_hbm, wq_hbm, wuk_hbm, wuv_hbm, wo_hbm, wr_hbm, wg_hbm,
            wu_hbm, wd_hbm, c_hbm, wmod_hbm, out_hbm,
            x_v, ckv_v, wq_v, wuk_v, wuv_v, wo_v, wr_v, wg_v, wu_v, wd_v, c_v,
            wmod_v, out_v, wq2_v, k_v, v_v, ctx_v, h_v, x1_v, h2_v, tmp_v, in_sems,
            out_sems, fix_sems, *, S, M, H, D, Dc):
    ng = H // _HG
    copies = {}

    def fetch(name, src, dst):
        copies[name] = pltpu.make_async_copy(src, dst, in_sems.at[len(copies)])
        copies[name].start()

    def fetch_group(name, src, dst, g):
        fetch((name, g), src.at[:, pl.ds(g * _HG, _HG), :], dst.at[g])

    ckv_spans = _spans(_CKV_ROWS)
    fetch_group("wuk", wuk_hbm, wuk_v, 0)
    for a, n in ckv_spans:
        fetch(("ckv", a), ckv_hbm.at[pl.ds(a, n), :], ckv_v.at[pl.ds(a, n), :])
    fetch_group("wuv", wuv_hbm, wuv_v, 0)
    fetch("c", c_hbm, c_v)
    fetch("wmod", wmod_hbm, wmod_v)
    fetch("x", x_hbm, x_v)
    for g in range(1, ng):
        fetch_group("wuk", wuk_hbm, wuk_v, g)
        fetch_group("wuv", wuv_hbm, wuv_v, g)
    for g in range(ng):
        fetch_group("wq", wq_hbm, wq_v, g)
    for name, src, dst in (("wo", wo_hbm, wo_v), ("wr", wr_hbm, wr_v), ("wg", wg_hbm, wg_v),
                           ("wu", wu_hbm, wu_v), ("wd", wd_hbm, wd_v)):
        fetch(name, src, dst)

    side_jobs = []

    def up_project(w, o_v, g, a, n):
        for e0 in range(0, _HG, 4):
            for r0 in range(a, a + n, _KVR):
                rows = min(_KVR, a + n - r0)
                r = jnp.dot(ckv_v[r0:r0 + rows, :], w[:, e0 * D:(e0 + 4) * D],
                            preferred_element_type=F32)
                for e in range(4):
                    o_v[g * _HG + e0 + e, r0 // 2:(r0 + rows) // 2, :] = _pack(
                        r[:, e * D:(e + 1) * D])
                if side_jobs:
                    side_jobs.pop(0)(r[0:8, 0:128])

    copies["wuk", 0].wait()
    for a, n in ckv_spans:
        copies["ckv", a].wait()
        if a == 0:
            w = wuk_v[0].reshape(Dc, _HG * D)
        if a == ckv_spans[-1][0]:
            copies["wuv", 0].wait()
        up_project(w, k_v, 0, a, n)
    up_project(wuv_v[0].reshape(Dc, _HG * D), v_v, 0, 0, S)

    for name in ("c", "wmod", "x", ("wuk", 1), ("wuv", 1)):
        copies[name].wait()
    cf = c_v[...].astype(F32)
    sc = jnp.broadcast_to(cf * jax.nn.sigmoid(cf), (16, M)).astype(BF16)
    mod = _rnd(jnp.dot(sc, wmod_v[...], preferred_element_type=F32)[0:1, :])
    sa, ca, ga, sb, cb, gb = (mod[:, i * M:(i + 1) * M] for i in range(6))

    def x_rows(a, n, anchor):
        return _unpack(_after(pltpu.bitcast(x_v[a:a + n, :], U32), anchor)).astype(F32)

    def first_adaln(a, n, anchor):
        h_v[a // 2:(a + n) // 2, :] = _pack(_adaln(x_rows(a, n, anchor), sa, ca))

    def regroup_wq(t, a, n, anchor):
        tmp_v[...] = _after(pltpu.bitcast(wq_v[t, a:a + n].reshape(n * _HG, D), U32), anchor)
        for e in range(_HG // 2):
            w = tmp_v[pl.ds(e, n, stride=_HG // 2), :]
            dst = wq2_v.at[t * (_HG // 2) + e]
            dst[a // 2:(a + n) // 2, 0:D] = _pack(pltpu.bitcast(w << 16, F32))
            dst[a // 2:(a + n) // 2, D:2 * D] = _pack(
                pltpu.bitcast(w & jnp.uint32(0xFFFF0000), F32))

    side_jobs += [functools.partial(first_adaln, a, _LNR) for a in range(0, S, _LNR)]
    side_jobs += [functools.partial(regroup_wq, t, a, 128)
                  for t in range(ng) for a in range(0, M, 128)]
    for g in range(1, ng):
        if g == 2:
            for name in copies:
                if name[0] in ("wuk", "wuv") and name[1] >= 2 or name[0] == "wq":
                    copies[name].wait()
        up_project(wuk_v[g].reshape(Dc, _HG * D), k_v, g, 0, S)
        up_project(wuv_v[g].reshape(Dc, _HG * D), v_v, g, 0, S)
    assert not side_jobs

    qscale = float(D ** -0.5 * math.log2(math.e))
    neg = float(-1e9 * math.log2(math.e))
    nb = S // _BQ
    hb = _BQ // 2

    def attn_body(j, bad):
        causal = (lax.broadcasted_iota(I32, (_BQ, _BQ), 1)
                  <= lax.broadcasted_iota(I32, (_BQ, _BQ), 0))
        qs = {}

        def q_project(c):
            hc = _unpack(h_v[c * _QC // 2:(c + 1) * _QC // 2, :])
            q = jnp.dot(hc, _unpack(wq2_v[j]), preferred_element_type=F32) * qscale
            for e in range(2):
                for t in range(_QC // _BQ):
                    qs[e, c * _QC // _BQ + t] = (
                        q[t * _BQ:(t + 1) * _BQ, e * D:(e + 1) * D].astype(BF16))

        def scores(e, i):
            n = i * _BQ
            k = _unpack(k_v[2 * j + e, 0:(i + 1) * hb, :])
            s = lax.dot_general(qs.pop((e, i)), k, _NT, preferred_element_type=F32)
            sd = jnp.where(causal, s[:, n:], neg)
            return jnp.concatenate([s[:, :n], sd], axis=1) if n else sd

        def context(e, i, s, bad):
            p = jnp.exp2(s)
            l = jnp.sum(p, axis=1, keepdims=True)
            v = _unpack(v_v[2 * j + e, 0:(i + 1) * hb, :])
            o = jnp.dot(p.astype(BF16), v, preferred_element_type=F32)
            ctx_v[2 * j + e, i * hb:(i + 1) * hb, :] = _pack(o * (1.0 / l))
            mag = jnp.abs(o)
            safe = ((l >= 2.0 ** -_SUM_EXP) & (l <= 2.0 ** _SUM_EXP) & (mag < jnp.inf)
                    & ((l >= 1.0) | (mag >= 2.0 ** -_ACC_EXP)))
            for t in range(0, _BQ, 8):
                bad = jnp.where(safe[t:t + 8, :], bad, 1.0)
            return bad

        seq = [(e, i) for t in range(nb // 2) for e in range(2) for i in (t, nb // 2 + t)]
        projected, pending = [], None
        for t, (e, i) in enumerate(seq):
            for _, i2 in seq[t:t + 3]:
                if i2 * _BQ // _QC not in projected:
                    projected.append(i2 * _BQ // _QC)
                    q_project(projected[-1])
            s = scores(e, i)
            if pending is not None:
                bad = context(*pending, bad)
            pending = (e, i, s)
        return context(*pending, bad)

    with jax.named_scope('p2'):
        bad = lax.fori_loop(0, H // 2, attn_body, jnp.zeros((8, D), F32))

    @pl.when(jnp.max(bad) > 0.0)
    def _true_max_attention():
        def body(t, carry):
            j, b = t // (S // _FQ), t % (S // _FQ)
            rows = pl.ds(pl.multiple_of(b * (_FQ // 2), _FQ // 2), _FQ // 2)
            q = jnp.dot(_unpack(h_v[rows, :]), _unpack(wq2_v[j]),
                        preferred_element_type=F32) * qscale
            causal = (lax.broadcasted_iota(I32, (_FQ, S), 1)
                      <= lax.broadcasted_iota(I32, (_FQ, S), 0) + b * _FQ)
            for e in range(2):
                s = lax.dot_general(q[:, e * D:(e + 1) * D].astype(BF16),
                                    _unpack(k_v[2 * j + e]), _NT, preferred_element_type=F32)
                s = jnp.where(causal, s, neg)
                p = jnp.exp2(s - jnp.max(s, axis=1, keepdims=True))
                p = p * (1.0 / jnp.sum(p, axis=1, keepdims=True))
                ctx_v[2 * j + e, rows, :] = _pack(jnp.dot(
                    p.astype(BF16), _unpack(v_v[2 * j + e]), preferred_element_type=F32))
            return carry

        lax.fori_loop(0, (H // 2) * (S // _FQ), body, 0)

    for name in ("wo", "wr", "wg", "wu", "wd"):
        copies[name].wait()
    wrf = wr_v[...].astype(F32).reshape(1, M)
    wr = jnp.broadcast_to(wrf, (16, M)).astype(BF16)
    out_spans = _spans(_OUT_ROWS)
    out_copies, scores_r = [], []

    def second_adaln(a, att, h2_rows, anchor):
        n = att.shape[0]
        att = pltpu.bitcast(_after(pltpu.bitcast(att, U32), anchor), F32)
        x1 = _rnd(x_rows(a, n, anchor) + _rnd(ga * _rnd(att)))
        h2 = _adaln(x1, sb, cb)
        x1_v[a:a + n, :] = x1
        h2_v[a:a + n, :] = h2
        out_v[a:a + n, :] = (x1 + _rnd(gb * (h2 + h2 * 0.0))).astype(BF16)
        h2_rows.append(h2.astype(BF16))

    def route_and_flush(a, n, h2_rows):
        r = lax.dot_general(wr, jnp.concatenate(h2_rows, axis=0), _NT,
                            preferred_element_type=F32)
        scores_r.extend(r[0:8, t:t + 128] for t in range(0, n, 128))
        out_copies.append(pltpu.make_async_copy(
            out_v.at[pl.ds(a, n), :], out_hbm.at[pl.ds(a, n), :], out_sems.at[len(out_copies)]))
        out_copies[-1].start()

    flush = None
    for a, n in out_spans:
        steps = [(c0, r0) for c0 in range(0, M, 128) for r0 in range(a, a + n, _OR)]
        per_step = -(-len(side_jobs) // max(len(steps) - 1, 1))
        parts = {}
        for c0, r0 in steps:
            rows = min(_OR, a + n - r0)
            ctx = jnp.concatenate(
                [_unpack(ctx_v[h, r0 // 2:(r0 + rows) // 2, :]) for h in range(H)], axis=1)
            parts[c0, r0] = jnp.dot(ctx, wo_v[:, c0:c0 + 128], preferred_element_type=F32)
            for _ in range(min(per_step, len(side_jobs))):
                side_jobs.pop(0)(parts[c0, r0][0:8, :])
        if flush is not None:
            flush()
        att = jnp.concatenate(
            [jnp.concatenate([parts[c0, r0] for r0 in range(a, a + n, _OR)], axis=0)
             for c0 in range(0, M, 128)], axis=1)
        h2_rows = []
        side_jobs += [functools.partial(second_adaln, a + t, att[t:t + _LNR, :], h2_rows)
                      for t in range(0, n, _LNR)]
        flush = functools.partial(route_and_flush, a, n, h2_rows)
    while side_jobs:
        side_jobs.pop(0)(att[0:8, 0:128])
    flush()

    sub8 = lax.broadcasted_iota(I32, (8, 128), 0)
    tiles = []
    for t in range(0, len(scores_r), 8):
        r = scores_r[t]
        for u in range(1, 8):
            r = jnp.where(sub8 == u, scores_r[t + u], r)
        tiles.append(r)
    r = _rnd(jnp.concatenate(tiles, axis=0))
    tok = lax.broadcasted_iota(I32, r.shape, 0) * 128 + lax.broadcasted_iota(I32, r.shape, 1)
    bits = pltpu.bitcast(jnp.where(r == 0.0, 0.0, r), I32) >> 16
    order = jnp.where(bits < 0, -(bits & 0x7FFF), bits) + 0x8000
    order = jnp.where(r != r, 0, order)
    key = pltpu.bitcast((order * S + (S - 1 - tok)) + 0x20000000, F32)
    idx = []
    for _ in range(_TOPC):
        top = jnp.max(jnp.max(key, axis=0, keepdims=True), axis=1, keepdims=True)
        idx.append((S - 1) - (pltpu.bitcast(top, I32)[0, 0] & (S - 1)))
        key = jnp.where(key == top, 0.0, key)

    hs = jnp.concatenate([h2_v[pl.ds(i, 1), :] for i in idx], axis=0)
    xs = jnp.concatenate([x1_v[pl.ds(i, 1), :] for i in idx], axis=0)
    hs16 = jnp.concatenate([hs, hs], axis=0).astype(BF16)
    g = _rnd(lax.dot_general(hs16, wg_v[...], _NT, preferred_element_type=F32))
    u = _rnd(lax.dot_general(hs16, wu_v[...], _NT, preferred_element_type=F32))
    act = (_rnd(g * jax.nn.sigmoid(g)) * u).astype(BF16)
    y = _rnd(jnp.dot(act, wd_v[...], preferred_element_type=F32))[0:_TOPC, :]
    rs = _rnd(jnp.sum(hs * wrf, axis=1, keepdims=True))
    y = _rnd(y * _rnd(jax.nn.sigmoid(rs)))
    new = xs + _rnd(gb * _rnd(hs + _rnd(hs * 0.0 + y)))

    for cp in out_copies:
        cp.wait()
    sub16 = lax.broadcasted_iota(I32, (16, M), 0)
    groups = [pl.ds(pl.multiple_of((i // 16) * 16, 16), 16) for i in idx]
    for n, i in enumerate(idx):
        old = out_v[groups[n], :].astype(F32)
        out_v[groups[n], :] = jnp.where(sub16 == i % 16, new[n:n + 1, :], old).astype(BF16)
    fixes = []
    for n, i in enumerate(idx):
        first = True
        for prev in idx[:n]:
            first = (prev // 16 != i // 16) & first
        fixes.append((first, pltpu.make_async_copy(
            out_v.at[groups[n], :], out_hbm.at[groups[n], :], fix_sems.at[n])))
    for first, cp in fixes:
        pl.when(first)(cp.start)
    for first, cp in fixes:
        pl.when(first)(cp.wait)


@jax.jit
def pallas_adaLN_cond__compressed_kv_cla__moe_arch_mod__prompt_kernel(
    A_x: jax.Array,
    A_c_kv: jax.Array,
    A_w_q: jax.Array,
    A_w_uk: jax.Array,
    A_w_uv: jax.Array,
    A_w_o: jax.Array,
    B_x: jax.Array,
    B_w_r: jax.Array,
    B_w_gate: jax.Array,
    B_w_up: jax.Array,
    B_w_down: jax.Array,
    c: jax.Array,
    w_mod: jax.Array,
):
    del B_x
    B, S, M = A_x.shape
    Dc = A_c_kv.shape[2]
    _, H, D = A_w_q.shape
    assert B == 1 and A_c_kv.shape[1] == S == sum(_CKV_ROWS) == sum(_OUT_ROWS)

    args = (
        A_x.reshape(S, M), A_c_kv.reshape(S, Dc), A_w_q, A_w_uk, A_w_uv,
        A_w_o.reshape(H * D, M), B_w_r, B_w_gate.T, B_w_up.T, B_w_down, c, w_mod,
    )
    ng = H // _HG
    scratch = [
        pltpu.VMEM((ng, a.shape[0], _HG, D) if a.ndim == 3 else a.shape, a.dtype)
        for a in args
    ] + [
        pltpu.VMEM((S, M), BF16),
        pltpu.VMEM((H // 2, M // 2, 2 * D), U32),
        pltpu.VMEM((H, S // 2, D), U32),
        pltpu.VMEM((H, S // 2, D), U32),
        pltpu.VMEM((H, S // 2, D), U32),
        pltpu.VMEM((S // 2, M), U32),
        pltpu.VMEM((S, M), F32),
        pltpu.VMEM((S, M), F32),
        pltpu.VMEM((128 * _HG // 2, D), U32),
        pltpu.SemaphoreType.DMA((3 * ng + len(_CKV_ROWS) + 8,)),
        pltpu.SemaphoreType.DMA((len(_OUT_ROWS),)),
        pltpu.SemaphoreType.DMA((_TOPC,)),
    ]

    def kernel_function(*refs):
        _kernel(*refs, S=S, M=M, H=H, D=D, Dc=Dc)

    out = pl.pallas_call(
        kernel_function,
        in_specs=[pl.BlockSpec(memory_space=pltpu.HBM)] * len(args),
        out_specs=pl.BlockSpec(memory_space=pltpu.HBM),
        out_shape=jax.ShapeDtypeStruct((S, M), A_x.dtype),
        scratch_shapes=scratch,
        compiler_params=pltpu.CompilerParams(vmem_limit_bytes=120 * 1024 * 1024),
        name="adaln_cla_mod",
    )(*args)
    return out.reshape(B, S, M)
```

```python
import functools
import math

import jax
import jax.numpy as jnp
from jax import lax
import jax.experimental.pallas as pl
import jax.experimental.pallas.tpu as pltpu

F32 = jnp.float32
BF16 = jnp.bfloat16
U32 = jnp.uint32
I32 = jnp.int32

_NT = (((1,), (1,)), ((), ()))
_EPS = 1e-5
_TOPC = 8
_BQ = 128
_QC = 256
_HG = 8
_KVR = 256
_LNR = 16
_RGR = 32
_OH = 8
_OR = 128
_FQ = 256
_TINY = 2.0 ** -60
_CKV_ROWS = (256, 768, 1024)
_OUT_ROWS = (1536, 512)


def _rnd(v):
    return v.astype(BF16).astype(F32)


def _adaln(x, shift, scale):
    mean = jnp.mean(x, axis=1, keepdims=True)
    d = x - mean
    var = _rnd(jnp.mean(d * d, axis=1, keepdims=True))
    den = _rnd(jnp.sqrt(_rnd(var + _rnd(jnp.full((1, 1), _EPS, F32)))))
    n = _rnd(_rnd(x - _rnd(mean)) / den)
    return _rnd(_rnd(n * _rnd(1.0 + scale)) + shift)


def _pack(v):
    return pltpu.bitcast(v.astype(BF16), U32)


def _unpack(v):
    return pltpu.bitcast(v, BF16)


def _after(words, anchor):
    zero = jnp.where(anchor * anchor < 0.0, jnp.uint32(1), jnp.uint32(0))
    return words | jnp.tile(zero, (words.shape[0] // 8, words.shape[1] // 128))


def _spans(sizes):
    out, start = [], 0
    for n in sizes:
        out.append((start, n))
        start += n
    return out


def _kernel(x_hbm, ckv_hbm, wq_hbm, wuk_hbm, wuv_hbm, wo_hbm, wr_hbm, wg_hbm,
            wu_hbm, wd_hbm, c_hbm, wmod_hbm, out_hbm,
            x_v, ckv_v, wq_v, wuk_v, wuv_v, wo_v, wr_v, wg_v, wu_v, wd_v, c_v,
            wmod_v, out_v, wq2_v, k_v, v_v, ctx_v, h_v, x1_v, h2_v, tmp_v, wkv_v, col_v, mod_v, in_sems,
            out_sems, fix_sems, *, S, M, H, D, Dc):
    ng = H // _HG
    copies = {}

    def fetch(name, src, dst):
        copies[name] = pltpu.make_async_copy(src, dst, in_sems.at[len(copies)])
        copies[name].start()

    def fetch_group(name, src, dst, g):
        fetch((name, g), src.at[:, pl.ds(g * _HG, _HG), :], dst.at[g])

    ckv_spans = _spans(_CKV_ROWS)
    fetch_group("wuk", wuk_hbm, wuk_v, 0)
    for a, n in ckv_spans:
        fetch(("ckv", a), ckv_hbm.at[pl.ds(a, n), :], ckv_v.at[pl.ds(a, n), :])
    fetch_group("wuv", wuv_hbm, wuv_v, 0)
    fetch_group("wuk", wuk_hbm, wuk_v, 1)
    fetch_group("wuv", wuv_hbm, wuv_v, 1)
    fetch("c", c_hbm, c_v)
    fetch("wmod", wmod_hbm, wmod_v)
    fetch("x", x_hbm, x_v)
    for g in range(2, ng):
        fetch_group("wuk", wuk_hbm, wuk_v, g)
        fetch_group("wuv", wuv_hbm, wuv_v, g)
    for g in range(ng):
        fetch_group("wq", wq_hbm, wq_v, g)
    for name, src, dst in (("wo", wo_hbm, wo_v), ("wr", wr_hbm, wr_v), ("wg", wg_hbm, wg_v),
                           ("wu", wu_hbm, wu_v), ("wd", wd_hbm, wd_v)):
        fetch(name, src, dst)

    def regroup(src, g, dst, a, anchor):
        n = _RGR
        tmp_v[...] = _after(pltpu.bitcast(src[g, a:a + n].reshape(n * _HG, D), U32), anchor)
        for e in range(_HG // 2):
            w = tmp_v[pl.ds(e, n, stride=_HG // 2), :]
            dst(e)[a // 2:(a + n) // 2, 0:D] = _pack(pltpu.bitcast(w << 16, F32))
            dst(e)[a // 2:(a + n) // 2, D:2 * D] = _pack(
                pltpu.bitcast(w & jnp.uint32(0xFFFF0000), F32))

    def silu_column(anchor):
        del anchor
        cf = c_v[...].astype(F32)
        sc = _rnd(cf * jax.nn.sigmoid(cf))
        col_v[...] = jnp.broadcast_to(sc, (128, M)).T

    def modulation(t, anchor):
        w = _unpack(_after(pltpu.bitcast(wmod_v[:, t:t + 128], U32), anchor)).astype(F32)
        mod_v[t // M:t // M + 1, t % M:t % M + 128] = _rnd(
            jnp.sum(w * col_v[...], axis=0, keepdims=True))

    def x_rows(a, n, anchor):
        return _unpack(_after(pltpu.bitcast(x_v[a:a + n, :], U32), anchor)).astype(F32)

    def first_adaln(a, anchor):
        h = _adaln(x_rows(a, _LNR, anchor), mod_v[0:1, :], mod_v[1:2, :])
        h_v[a // 2:(a + _LNR) // 2, :] = _pack(h)

    stages = [(src, g, o_v) for g in range(ng) for src, o_v in ((wuk_v, k_v), (wuv_v, v_v))]
    early = [silu_column]
    for t in range(0, 6 * M, 128):
        early += [functools.partial(modulation, t), None, None]
    late = [functools.partial(first_adaln, a) for a in range(0, S, _LNR)]
    late += [functools.partial(regroup, wq_v, g, lambda e, g=g: wq2_v.at[g * (_HG // 2) + e], a)
             for g in range(ng) for a in range(0, M, _RGR)]
    jobs = []
    copies["wuk", 0].wait()
    for t, (src, g, o_v) in enumerate(stages):
        for r0 in range(0, S, _KVR):
            if t == 0 and ("ckv", r0) in copies:
                copies["ckv", r0].wait()
                if r0 == 0:
                    w0 = src[g].reshape(Dc, _HG * D)
            if r0 == S // 2 and t + 1 < len(stages):
                if t == 0:
                    copies["wuv", 0].wait()
                elif t == 1:
                    for name in (("wuk", 1), ("wuv", 1), "c", "wmod"):
                        copies[name].wait()
                    jobs += early
                elif t == 3:
                    for name in copies:
                        if name[0] in ("wuk", "wuv") and name[1] >= 2 or name[0] in ("wq", "x"):
                            copies[name].wait()
                    jobs += late
                nsrc, ngrp, _ = stages[t + 1]
                jobs[0:0] = [
                    functools.partial(regroup, nsrc, ngrp,
                                      lambda e, t=t: wkv_v.at[(t + 1) % 2, e], a)
                    for a in range(0, Dc, _RGR)]
            for e0 in range(0, _HG, 4):
                if t == 0:
                    w = w0[:, e0 * D:(e0 + 4) * D]
                else:
                    w = jnp.concatenate(
                        [_unpack(wkv_v[t % 2, e0 // 2 + e]) for e in range(2)], axis=1)
                r = jnp.dot(ckv_v[r0:r0 + _KVR, :], w, preferred_element_type=F32)
                for e in range(4):
                    o_v[g * _HG + e0 + e, r0 // 2:(r0 + _KVR) // 2, :] = _pack(
                        r[:, e * D:(e + 1) * D])
                    job = jobs.pop(0) if jobs else None
                    if job is not None:
                        job(r[0:8, e * D:(e + 1) * D])
    assert not jobs

    qscale = float(D ** -0.5 * math.log2(math.e))
    neg = float(-1e9 * math.log2(math.e))
    nb = S // _BQ
    hb = _BQ // 2

    def attn_body(j, seen):
        causal = (lax.broadcasted_iota(I32, (_BQ, _BQ), 1)
                  <= lax.broadcasted_iota(I32, (_BQ, _BQ), 0))
        qs = {}

        def q_project(c):
            hc = _unpack(h_v[c * _QC // 2:(c + 1) * _QC // 2, :])
            q = jnp.dot(hc, _unpack(wq2_v[j]), preferred_element_type=F32) * qscale
            for e in range(2):
                for t in range(_QC // _BQ):
                    qs[e, c * _QC // _BQ + t] = (
                        q[t * _BQ:(t + 1) * _BQ, e * D:(e + 1) * D].astype(BF16))

        def scores(e, i):
            n = i * _BQ
            k = _unpack(k_v[2 * j + e, 0:(i + 1) * hb, :])
            s = lax.dot_general(qs.pop((e, i)), k, _NT, preferred_element_type=F32)
            sd = jnp.where(causal, s[:, n:], neg)
            return jnp.concatenate([s[:, :n], sd], axis=1) if n else sd

        def context(e, i, s, seen):
            p = jnp.exp2(s)
            l = jnp.sum(p, axis=1, keepdims=True)
            v = _unpack(v_v[2 * j + e, 0:(i + 1) * hb, :])
            o = jnp.dot(p.astype(BF16), v, preferred_element_type=F32)
            ctx_v[2 * j + e, i * hb:(i + 1) * hb, :] = _pack(o * (1.0 / l))
            mag = jnp.maximum(jnp.abs(o), l * _TINY)
            l = jnp.broadcast_to(l, mag.shape)
            mag_lo, mag_hi, l_lo = seen
            for t in range(0, _BQ, 8):
                mag_lo = jnp.minimum(mag_lo, mag[t:t + 8, :])
                mag_hi = jnp.maximum(mag_hi, mag[t:t + 8, :])
                l_lo = jnp.minimum(l_lo, l[t:t + 8, :])
            return mag_lo, mag_hi, l_lo

        seq = [(e, i) for t in range(nb // 2) for e in range(2) for i in (t, nb - 1 - t)]
        projected, pending = [], None
        for t, (e, i) in enumerate(seq):
            for _, i2 in seq[t:t + 3]:
                if i2 * _BQ // _QC not in projected:
                    projected.append(i2 * _BQ // _QC)
                    q_project(projected[-1])
            s = scores(e, i)
            if pending is not None:
                seen = context(*pending, seen)
            pending = (e, i, s)
        return context(*pending, seen)

    ones = jnp.ones((8, D), F32)
    mag_lo, mag_hi, l_lo = lax.fori_loop(0, H // 2, attn_body, (ones, ones, ones))
    safe = (mag_hi <= 1.0 / _TINY) & (l_lo >= _TINY) & (mag_lo >= _TINY)

    @pl.when(jnp.max(jnp.where(safe, 0.0, 1.0)) > 0.0)
    def _true_max_attention():
        def body(t, carry):
            j, b = t // (S // _FQ), t % (S // _FQ)
            rows = pl.ds(pl.multiple_of(b * (_FQ // 2), _FQ // 2), _FQ // 2)
            q = jnp.dot(_unpack(h_v[rows, :]), _unpack(wq2_v[j]),
                        preferred_element_type=F32) * qscale
            causal = (lax.broadcasted_iota(I32, (_FQ, S), 1)
                      <= lax.broadcasted_iota(I32, (_FQ, S), 0) + b * _FQ)
            for e in range(2):
                s = lax.dot_general(q[:, e * D:(e + 1) * D].astype(BF16),
                                    _unpack(k_v[2 * j + e]), _NT, preferred_element_type=F32)
                s = jnp.where(causal, s, neg)
                p = jnp.exp2(s - jnp.max(s, axis=1, keepdims=True))
                p = p * (1.0 / jnp.sum(p, axis=1, keepdims=True))
                ctx_v[2 * j + e, rows, :] = _pack(jnp.dot(
                    p.astype(BF16), _unpack(v_v[2 * j + e]), preferred_element_type=F32))
            return carry

        lax.fori_loop(0, (H // 2) * (S // _FQ), body, 0)

    for name in ("wo", "wr", "wg", "wu", "wd"):
        copies[name].wait()
    wrf = wr_v[...].astype(F32).reshape(1, M)
    lane = lax.broadcasted_iota(I32, (8, 128), 1)
    tiles = [jnp.zeros((8, 128), F32) for _ in range(S // 1024)]

    def second_adaln(a, att, anchor):
        att = pltpu.bitcast(_after(pltpu.bitcast(att, U32), anchor), F32)
        x1 = _rnd(x_rows(a, _LNR, anchor) + _rnd(mod_v[2:3, :] * _rnd(att)))
        h2 = _adaln(x1, mod_v[3:4, :], mod_v[4:5, :])
        x1_v[a:a + _LNR, :] = x1
        h2_v[a:a + _LNR, :] = h2
        out_v[a:a + _LNR, :] = (x1 + _rnd(mod_v[5:6, :] * (h2 + h2 * 0.0))).astype(BF16)
        r = jnp.sum(h2 * wrf, axis=1, keepdims=True)
        for u in range(0, _LNR, 8):
            t, ln = divmod((a + u) // 8, 128)
            tiles[t] = jnp.where(lane == ln, r[u:u + 8, :], tiles[t])

    out_copies = [
        pltpu.make_async_copy(out_v.at[pl.ds(a, n), :], out_hbm.at[pl.ds(a, n), :], out_sems.at[i])
        for i, (a, n) in enumerate(_spans(_OUT_ROWS))]
    for r0 in range(0, S, _OR):
        if r0 == _OUT_ROWS[0] + _OR:
            out_copies[0].start()
        parts = []
        for c0 in range(0, M, 128):
            acc = None
            for h0 in range(0, H, _OH):
                ctx = jnp.concatenate([_unpack(ctx_v[h, r0 // 2:(r0 + _OR) // 2, :])
                                       for h in range(h0, h0 + _OH)], axis=1)
                part = jnp.dot(ctx, wo_v[h0 * D:(h0 + _OH) * D, c0:c0 + 128],
                               preferred_element_type=F32)
                acc = part if acc is None else acc + part
                if jobs:
                    jobs.pop(0)(part[0:8, :])
            parts.append(acc)
        assert not jobs
        att = jnp.concatenate(parts, axis=1)
        jobs = [functools.partial(second_adaln, r0 + t, att[t:t + _LNR, :])
                for t in range(0, _OR, _LNR)]
    for job in jobs:
        job(att[0:8, 0:128])
    out_copies[1].start()

    r = _rnd(jnp.concatenate(tiles, axis=0))
    sub = lax.broadcasted_iota(I32, r.shape, 0)
    tok = (sub // 8) * 1024 + lax.broadcasted_iota(I32, r.shape, 1) * 8 + sub % 8
    bits = pltpu.bitcast(jnp.where(r == 0.0, 0.0, r), I32) >> 16
    order = jnp.where(bits < 0, -(bits & 0x7FFF), bits) + 0x8000
    order = jnp.where(r != r, 0, order)
    key = pltpu.bitcast((order * S + (S - 1 - tok)) + 0x20000000, F32)
    idx = []
    for _ in range(_TOPC):
        top = jnp.max(jnp.max(key, axis=0, keepdims=True), axis=1, keepdims=True)
        idx.append((S - 1) - (pltpu.bitcast(top, I32)[0, 0] & (S - 1)))
        key = jnp.where(key == top, 0.0, key)

    hs = jnp.concatenate([h2_v[pl.ds(i, 1), :] for i in idx], axis=0)
    xs = jnp.concatenate([x1_v[pl.ds(i, 1), :] for i in idx], axis=0)
    hs16 = jnp.concatenate([hs, hs], axis=0).astype(BF16)
    g = _rnd(lax.dot_general(hs16, wg_v[...], _NT, preferred_element_type=F32))
    u = _rnd(lax.dot_general(hs16, wu_v[...], _NT, preferred_element_type=F32))
    act = (_rnd(g * jax.nn.sigmoid(g)) * u).astype(BF16)
    y = _rnd(jnp.dot(act, wd_v[...], preferred_element_type=F32))[0:_TOPC, :]
    rs = _rnd(jnp.sum(hs * wrf, axis=1, keepdims=True))
    y = _rnd(y * _rnd(jax.nn.sigmoid(rs)))
    new = xs + _rnd(mod_v[5:6, :] * _rnd(hs + _rnd(hs * 0.0 + y)))

    for cp in out_copies:
        cp.wait()
    sub16 = lax.broadcasted_iota(I32, (16, M), 0)
    groups = [pl.ds(pl.multiple_of((i // 16) * 16, 16), 16) for i in idx]
    for n, i in enumerate(idx):
        old = out_v[groups[n], :].astype(F32)
        out_v[groups[n], :] = jnp.where(sub16 == i % 16, new[n:n + 1, :], old).astype(BF16)
    fixes = []
    for n, i in enumerate(idx):
        first = True
        for prev in idx[:n]:
            first = (prev // 16 != i // 16) & first
        fixes.append((first, pltpu.make_async_copy(
            out_v.at[groups[n], :], out_hbm.at[groups[n], :], fix_sems.at[n])))
    for first, cp in fixes:
        pl.when(first)(cp.start)
    for first, cp in fixes:
        pl.when(first)(cp.wait)


@jax.jit
def pallas_adaLN_cond__compressed_kv_cla__moe_arch_mod__prompt_kernel(
    A_x: jax.Array,
    A_c_kv: jax.Array,
    A_w_q: jax.Array,
    A_w_uk: jax.Array,
    A_w_uv: jax.Array,
    A_w_o: jax.Array,
    B_x: jax.Array,
    B_w_r: jax.Array,
    B_w_gate: jax.Array,
    B_w_up: jax.Array,
    B_w_down: jax.Array,
    c: jax.Array,
    w_mod: jax.Array,
):
    del B_x
    B, S, M = A_x.shape
    Dc = A_c_kv.shape[2]
    _, H, D = A_w_q.shape
    assert B == 1 and A_c_kv.shape[1] == S == sum(_CKV_ROWS) == sum(_OUT_ROWS)

    args = (
        A_x.reshape(S, M), A_c_kv.reshape(S, Dc), A_w_q, A_w_uk, A_w_uv,
        A_w_o.reshape(H * D, M), B_w_r, B_w_gate.T, B_w_up.T, B_w_down, c, w_mod,
    )
    ng = H // _HG
    scratch = [
        pltpu.VMEM((ng, a.shape[0], _HG, D) if a.ndim == 3 else a.shape, a.dtype)
        for a in args
    ] + [
        pltpu.VMEM((S, M), BF16),
        pltpu.VMEM((H // 2, M // 2, 2 * D), U32),
        pltpu.VMEM((H, S // 2, D), U32),
        pltpu.VMEM((H, S // 2, D), U32),
        pltpu.VMEM((H, S // 2, D), U32),
        pltpu.VMEM((S // 2, M), U32),
        pltpu.VMEM((S, M), F32),
        pltpu.VMEM((S, M), F32),
        pltpu.VMEM((_RGR * _HG // 2, D), U32),
        pltpu.VMEM((2, _HG // 2, Dc // 2, 2 * D), U32),
        pltpu.VMEM((M, 128), F32),
        pltpu.VMEM((8, M), F32),
        pltpu.SemaphoreType.DMA((3 * ng + len(_CKV_ROWS) + 8,)),
        pltpu.SemaphoreType.DMA((len(_OUT_ROWS),)),
        pltpu.SemaphoreType.DMA((_TOPC,)),
    ]

    def kernel_function(*refs):
        _kernel(*refs, S=S, M=M, H=H, D=D, Dc=Dc)

    out = pl.pallas_call(
        kernel_function,
        in_specs=[pl.BlockSpec(memory_space=pltpu.HBM)] * len(args),
        out_specs=pl.BlockSpec(memory_space=pltpu.HBM),
        out_shape=jax.ShapeDtypeStruct((S, M), A_x.dtype),
        scratch_shapes=scratch,
        compiler_params=pltpu.CompilerParams(vmem_limit_bytes=120 * 1024 * 1024),
        name="adaln_cla_mod",
    )(*args)
    return out.reshape(B, S, M)
```

```python
import functools
import math

import jax
import jax.numpy as jnp
from jax import lax
import jax.experimental.pallas as pl
import jax.experimental.pallas.tpu as pltpu

F32 = jnp.float32
BF16 = jnp.bfloat16
U32 = jnp.uint32
I32 = jnp.int32

_NT = (((1,), (1,)), ((), ()))
_EPS = 1e-5
_TOPC = 8
_BQ = 128
_QC = 256
_HG = 8
_KVR = 256
_LNR = 16
_RGR = 32
_OH = 8
_OR = 128
_FQ = 256
_TINY = 2.0 ** -60
_CKV_ROWS = (256, 768, 1024)
_OUT_ROWS = (1536, 512)


def _rnd(v):
    return v.astype(BF16).astype(F32)


def _adaln(x, shift, scale):
    mean = jnp.mean(x, axis=1, keepdims=True)
    d = x - mean
    var = _rnd(jnp.mean(d * d, axis=1, keepdims=True))
    den = _rnd(jnp.sqrt(_rnd(var + _rnd(jnp.full((1, 1), _EPS, F32)))))
    n = _rnd(_rnd(x - _rnd(mean)) / den)
    return _rnd(_rnd(n * _rnd(1.0 + scale)) + shift)


def _pack(v):
    return pltpu.bitcast(v.astype(BF16), U32)


def _unpack(v):
    return pltpu.bitcast(v, BF16)


def _after(words, anchor):
    zero = jnp.where(anchor * anchor < 0.0, jnp.uint32(1), jnp.uint32(0))
    return words | jnp.tile(zero, (words.shape[0] // 8, words.shape[1] // 128))


def _spans(sizes):
    out, start = [], 0
    for n in sizes:
        out.append((start, n))
        start += n
    return out


def _kernel(x_hbm, ckv_hbm, wq_hbm, wuk_hbm, wuv_hbm, wo_hbm, wmod_hbm, wg_hbm,
            wu_hbm, wd_hbm, wr_hbm, c_hbm, out_hbm,
            k_v, v_v, ctx_v, h_v, wq2_v, wkv_v, x1_v, h2_v, out_v, tmp_v, col_v,
            x_v, ckv_v, wq_v, wuk_v, wuv_v, wo_v, wmod_v, wg_v, wu_v, wd_v, wr_v, c_v,
            mod_v, in_sems, out_sems, fix_sems, *, S, M, H, D, Dc):
    ng = H // _HG
    copies = {}

    def fetch(name, src, dst):
        copies[name] = pltpu.make_async_copy(src, dst, in_sems.at[len(copies)])
        copies[name].start()

    def fetch_group(name, src, dst, g):
        fetch((name, g), src.at[:, pl.ds(g * _HG, _HG), :], dst.at[g])

    ckv_spans = _spans(_CKV_ROWS)
    fetch_group("wuk", wuk_hbm, wuk_v, 0)
    for a, n in ckv_spans:
        fetch(("ckv", a), ckv_hbm.at[pl.ds(a, n), :], ckv_v.at[pl.ds(a, n), :])
    fetch_group("wuv", wuv_hbm, wuv_v, 0)
    fetch_group("wuk", wuk_hbm, wuk_v, 1)
    fetch_group("wuv", wuv_hbm, wuv_v, 1)
    fetch("c", c_hbm, c_v)
    fetch("wmod", wmod_hbm, wmod_v)
    fetch("x", x_hbm, x_v)
    for g in range(2, ng):
        fetch_group("wuk", wuk_hbm, wuk_v, g)
        fetch_group("wuv", wuv_hbm, wuv_v, g)
    for g in range(ng):
        fetch_group("wq", wq_hbm, wq_v, g)
    for name, src, dst in (("wo", wo_hbm, wo_v), ("wr", wr_hbm, wr_v), ("wg", wg_hbm, wg_v),
                           ("wu", wu_hbm, wu_v), ("wd", wd_hbm, wd_v)):
        fetch(name, src, dst)

    def regroup(src, g, dst, a, anchor):
        n = _RGR
        tmp_v[...] = _after(pltpu.bitcast(src[g, a:a + n].reshape(n * _HG, D), U32), anchor)
        for e in range(_HG // 2):
            w = tmp_v[pl.ds(e, n, stride=_HG // 2), :]
            dst(e)[a // 2:(a + n) // 2, 0:D] = _pack(pltpu.bitcast(w << 16, F32))
            dst(e)[a // 2:(a + n) // 2, D:2 * D] = _pack(
                pltpu.bitcast(w & jnp.uint32(0xFFFF0000), F32))

    def silu_column(anchor):
        del anchor
        cf = c_v[...].astype(F32)
        sc = _rnd(cf * jax.nn.sigmoid(cf))
        col_v[...] = jnp.broadcast_to(sc, (128, M)).T

    def modulation(t, anchor):
        w = _unpack(_after(pltpu.bitcast(wmod_v[:, t:t + 128], U32), anchor)).astype(F32)
        mod_v[t // M:t // M + 1, t % M:t % M + 128] = _rnd(
            jnp.sum(w * col_v[...], axis=0, keepdims=True))

    def x_rows(a, n, anchor):
        return _unpack(_after(pltpu.bitcast(x_v[a:a + n, :], U32), anchor)).astype(F32)

    def first_adaln(a, anchor):
        h = _adaln(x_rows(a, _LNR, anchor), mod_v[0:1, :], mod_v[1:2, :])
        h_v[a // 2:(a + _LNR) // 2, :] = _pack(h)

    stages = [(src, g, o_v) for g in range(ng) for src, o_v in ((wuk_v, k_v), (wuv_v, v_v))]
    early = [silu_column]
    for t in range(0, 6 * M, 128):
        early += [functools.partial(modulation, t), None, None]
    late = [functools.partial(first_adaln, a) for a in range(0, S, _LNR)]
    late += [functools.partial(regroup, wq_v, g, lambda e, g=g: wq2_v.at[g * (_HG // 2) + e], a)
             for g in range(ng) for a in range(0, M, _RGR)]
    jobs = []
    copies["wuk", 0].wait()
    for t, (src, g, o_v) in enumerate(stages):
        for r0 in range(0, S, _KVR):
            if t == 0 and ("ckv", r0) in copies:
                copies["ckv", r0].wait()
                if r0 == 0:
                    w0 = src[g].reshape(Dc, _HG * D)
            if r0 == S // 2 and t + 1 < len(stages):
                if t == 0:
                    copies["wuv", 0].wait()
                elif t == 1:
                    for name in (("wuk", 1), ("wuv", 1), "c", "wmod"):
                        copies[name].wait()
                    jobs += early
                elif t == 3:
                    for name in copies:
                        if name[0] in ("wuk", "wuv") and name[1] >= 2 or name[0] in ("wq", "x"):
                            copies[name].wait()
                    jobs += late
                nsrc, ngrp, _ = stages[t + 1]
                jobs[0:0] = [
                    functools.partial(regroup, nsrc, ngrp,
                                      lambda e, t=t: wkv_v.at[(t + 1) % 2, e], a)
                    for a in range(0, Dc, _RGR)]
            for e0 in range(0, _HG, 4):
                if t == 0:
                    w = w0[:, e0 * D:(e0 + 4) * D]
                else:
                    w = jnp.concatenate(
                        [_unpack(wkv_v[t % 2, e0 // 2 + e]) for e in range(2)], axis=1)
                r = jnp.dot(ckv_v[r0:r0 + _KVR, :], w, preferred_element_type=F32)
                for e in range(4):
                    o_v[g * _HG + e0 + e, r0 // 2:(r0 + _KVR) // 2, :] = _pack(
                        r[:, e * D:(e + 1) * D])
                    job = jobs.pop(0) if jobs else None
                    if job is not None:
                        job(r[0:8, e * D:(e + 1) * D])
    assert not jobs

    qscale = float(D ** -0.5 * math.log2(math.e))
    neg = float(-1e9 * math.log2(math.e))
    nb = S // _BQ
    hb = _BQ // 2

    def attn_body(j, seen):
        causal = (lax.broadcasted_iota(I32, (_BQ, _BQ), 1)
                  <= lax.broadcasted_iota(I32, (_BQ, _BQ), 0))
        qs = {}

        def q_project(c):
            hc = _unpack(h_v[c * _QC // 2:(c + 1) * _QC // 2, :])
            q = jnp.dot(hc, _unpack(wq2_v[j]), preferred_element_type=F32) * qscale
            for e in range(2):
                for t in range(_QC // _BQ):
                    qs[e, c * _QC // _BQ + t] = (
                        q[t * _BQ:(t + 1) * _BQ, e * D:(e + 1) * D].astype(BF16))

        def scores(e, i):
            n = i * _BQ
            k = _unpack(k_v[2 * j + e, 0:(i + 1) * hb, :])
            s = lax.dot_general(qs.pop((e, i)), k, _NT, preferred_element_type=F32)
            sd = jnp.where(causal, s[:, n:], neg)
            return jnp.concatenate([s[:, :n], sd], axis=1) if n else sd

        def context(e, i, s, seen):
            p = jnp.exp2(s)
            l = jnp.sum(p, axis=1, keepdims=True)
            v = _unpack(v_v[2 * j + e, 0:(i + 1) * hb, :])
            o = jnp.dot(p.astype(BF16), v, preferred_element_type=F32)
            ctx_v[2 * j + e, i * hb:(i + 1) * hb, :] = _pack(o * (1.0 / l))
            mag = jnp.maximum(jnp.abs(o), l * _TINY)
            l = jnp.broadcast_to(l, mag.shape)
            mag_lo, mag_hi, l_lo = seen
            for t in range(0, _BQ, 8):
                mag_lo = jnp.minimum(mag_lo, mag[t:t + 8, :])
                mag_hi = jnp.maximum(mag_hi, mag[t:t + 8, :])
                l_lo = jnp.minimum(l_lo, l[t:t + 8, :])
            return mag_lo, mag_hi, l_lo

        seq = [(e, i) for t in range(nb // 2) for e in range(2) for i in (t, nb - 1 - t)]
        projected, pending = [], None
        for t, (e, i) in enumerate(seq):
            for _, i2 in seq[t:t + 3]:
                if i2 * _BQ // _QC not in projected:
                    projected.append(i2 * _BQ // _QC)
                    q_project(projected[-1])
            s = scores(e, i)
            if pending is not None:
                seen = context(*pending, seen)
            pending = (e, i, s)
        return context(*pending, seen)

    ones = jnp.ones((8, D), F32)
    mag_lo, mag_hi, l_lo = lax.fori_loop(0, H // 2, attn_body, (ones, ones, ones))
    safe = (mag_hi <= 1.0 / _TINY) & (l_lo >= _TINY) & (mag_lo >= _TINY)

    @pl.when(jnp.max(jnp.where(safe, 0.0, 1.0)) > 0.0)
    def _true_max_attention():
        def body(t, carry):
            j, b = t // (S // _FQ), t % (S // _FQ)
            rows = pl.ds(pl.multiple_of(b * (_FQ // 2), _FQ // 2), _FQ // 2)
            q = jnp.dot(_unpack(h_v[rows, :]), _unpack(wq2_v[j]),
                        preferred_element_type=F32) * qscale
            causal = (lax.broadcasted_iota(I32, (_FQ, S), 1)
                      <= lax.broadcasted_iota(I32, (_FQ, S), 0) + b * _FQ)
            for e in range(2):
                s = lax.dot_general(q[:, e * D:(e + 1) * D].astype(BF16),
                                    _unpack(k_v[2 * j + e]), _NT, preferred_element_type=F32)
                s = jnp.where(causal, s, neg)
                p = jnp.exp2(s - jnp.max(s, axis=1, keepdims=True))
                p = p * (1.0 / jnp.sum(p, axis=1, keepdims=True))
                ctx_v[2 * j + e, rows, :] = _pack(jnp.dot(
                    p.astype(BF16), _unpack(v_v[2 * j + e]), preferred_element_type=F32))
            return carry

        lax.fori_loop(0, (H // 2) * (S // _FQ), body, 0)

    for name in ("wo", "wr", "wg", "wu", "wd"):
        copies[name].wait()
    wrf = wr_v[...].astype(F32).reshape(1, M)
    lane = lax.broadcasted_iota(I32, (8, 128), 1)
    tiles = [jnp.zeros((8, 128), F32) for _ in range(S // 1024)]

    def second_adaln(a, att, anchor):
        att = pltpu.bitcast(_after(pltpu.bitcast(att, U32), anchor), F32)
        x1 = _rnd(x_rows(a, _LNR, anchor) + _rnd(mod_v[2:3, :] * _rnd(att)))
        h2 = _adaln(x1, mod_v[3:4, :], mod_v[4:5, :])
        x1_v[a:a + _LNR, :] = x1
        h2_v[a:a + _LNR, :] = h2
        out_v[a:a + _LNR, :] = (x1 + _rnd(mod_v[5:6, :] * (h2 + h2 * 0.0))).astype(BF16)
        r = jnp.sum(h2 * wrf, axis=1, keepdims=True)
        for u in range(0, _LNR, 8):
            t, ln = divmod((a + u) // 8, 128)
            tiles[t] = jnp.where(lane == ln, r[u:u + 8, :], tiles[t])

    out_copies = [
        pltpu.make_async_copy(out_v.at[pl.ds(a, n), :], out_hbm.at[pl.ds(a, n), :], out_sems.at[i])
        for i, (a, n) in enumerate(_spans(_OUT_ROWS))]
    for r0 in range(0, S, _OR):
        if r0 == _OUT_ROWS[0] + _OR:
            out_copies[0].start()
        parts = []
        for c0 in range(0, M, 128):
            acc = None
            for h0 in range(0, H, _OH):
                ctx = jnp.concatenate([_unpack(ctx_v[h, r0 // 2:(r0 + _OR) // 2, :])
                                       for h in range(h0, h0 + _OH)], axis=1)
                part = jnp.dot(ctx, wo_v[h0 * D:(h0 + _OH) * D, c0:c0 + 128],
                               preferred_element_type=F32)
                acc = part if acc is None else acc + part
                if jobs:
                    jobs.pop(0)(part[0:8, :])
            parts.append(acc)
        assert not jobs
        att = jnp.concatenate(parts, axis=1)
        jobs = [functools.partial(second_adaln, r0 + t, att[t:t + _LNR, :])
                for t in range(0, _OR, _LNR)]
    for job in jobs:
        job(att[0:8, 0:128])
    out_copies[1].start()

    r = _rnd(jnp.concatenate(tiles, axis=0))
    sub = lax.broadcasted_iota(I32, r.shape, 0)
    tok = (sub // 8) * 1024 + lax.broadcasted_iota(I32, r.shape, 1) * 8 + sub % 8
    bits = pltpu.bitcast(jnp.where(r == 0.0, 0.0, r), I32) >> 16
    order = jnp.where(bits < 0, -(bits & 0x7FFF), bits) + 0x8000
    order = jnp.where(r != r, 0, order)
    key = pltpu.bitcast((order * S + (S - 1 - tok)) + 0x20000000, F32)
    idx = []
    for _ in range(_TOPC):
        top = jnp.max(jnp.max(key, axis=0, keepdims=True), axis=1, keepdims=True)
        idx.append((S - 1) - (pltpu.bitcast(top, I32)[0, 0] & (S - 1)))
        key = jnp.where(key == top, 0.0, key)

    hs = jnp.concatenate([h2_v[pl.ds(i, 1), :] for i in idx], axis=0)
    xs = jnp.concatenate([x1_v[pl.ds(i, 1), :] for i in idx], axis=0)
    hs16 = jnp.concatenate([hs, hs], axis=0).astype(BF16)
    g = _rnd(lax.dot_general(hs16, wg_v[...], _NT, preferred_element_type=F32))
    u = _rnd(lax.dot_general(hs16, wu_v[...], _NT, preferred_element_type=F32))
    act = (_rnd(g * jax.nn.sigmoid(g)) * u).astype(BF16)
    y = _rnd(jnp.dot(act, wd_v[...], preferred_element_type=F32))[0:_TOPC, :]
    rs = _rnd(jnp.sum(hs * wrf, axis=1, keepdims=True))
    y = _rnd(y * _rnd(jax.nn.sigmoid(rs)))
    new = xs + _rnd(mod_v[5:6, :] * _rnd(hs + _rnd(hs * 0.0 + y)))

    for cp in out_copies:
        cp.wait()
    sub16 = lax.broadcasted_iota(I32, (16, M), 0)
    groups = [pl.ds(pl.multiple_of((i // 16) * 16, 16), 16) for i in idx]
    for n, i in enumerate(idx):
        old = out_v[groups[n], :].astype(F32)
        out_v[groups[n], :] = jnp.where(sub16 == i % 16, new[n:n + 1, :], old).astype(BF16)
    fixes = []
    for n, i in enumerate(idx):
        first = True
        for prev in idx[:n]:
            first = (prev // 16 != i // 16) & first
        fixes.append((first, pltpu.make_async_copy(
            out_v.at[groups[n], :], out_hbm.at[groups[n], :], fix_sems.at[n])))
    for first, cp in fixes:
        pl.when(first)(cp.start)
    for first, cp in fixes:
        pl.when(first)(cp.wait)


@jax.jit
def pallas_adaLN_cond__compressed_kv_cla__moe_arch_mod__prompt_kernel(
    A_x: jax.Array,
    A_c_kv: jax.Array,
    A_w_q: jax.Array,
    A_w_uk: jax.Array,
    A_w_uv: jax.Array,
    A_w_o: jax.Array,
    B_x: jax.Array,
    B_w_r: jax.Array,
    B_w_gate: jax.Array,
    B_w_up: jax.Array,
    B_w_down: jax.Array,
    c: jax.Array,
    w_mod: jax.Array,
):
    del B_x
    B, S, M = A_x.shape
    Dc = A_c_kv.shape[2]
    _, H, D = A_w_q.shape
    assert B == 1 and A_c_kv.shape[1] == S == sum(_CKV_ROWS) == sum(_OUT_ROWS)

    args = (
        A_x.reshape(S, M), A_c_kv.reshape(S, Dc), A_w_q, A_w_uk, A_w_uv,
        A_w_o.reshape(H * D, M), w_mod, B_w_gate.T, B_w_up.T, B_w_down, B_w_r, c,
    )
    ng = H // _HG
    scratch = [
        pltpu.VMEM((H, S // 2, D), U32),
        pltpu.VMEM((H, S // 2, D), U32),
        pltpu.VMEM((H, S // 2, D), U32),
        pltpu.VMEM((S // 2, M), U32),
        pltpu.VMEM((H // 2, M // 2, 2 * D), U32),
        pltpu.VMEM((2, _HG // 2, Dc // 2, 2 * D), U32),
        pltpu.VMEM((S, M), F32),
        pltpu.VMEM((S, M), F32),
        pltpu.VMEM((S, M), BF16),
        pltpu.VMEM((_RGR * _HG // 2, D), U32),
        pltpu.VMEM((M, 128), F32),
    ] + [
        pltpu.VMEM((ng, a.shape[0], _HG, D) if a.ndim == 3 else a.shape, a.dtype)
        for a in args
    ] + [
        pltpu.VMEM((8, M), F32),
        pltpu.SemaphoreType.DMA((3 * ng + len(_CKV_ROWS) + 8,)),
        pltpu.SemaphoreType.DMA((len(_OUT_ROWS),)),
        pltpu.SemaphoreType.DMA((_TOPC,)),
    ]

    def kernel_function(*refs):
        _kernel(*refs, S=S, M=M, H=H, D=D, Dc=Dc)

    out = pl.pallas_call(
        kernel_function,
        in_specs=[pl.BlockSpec(memory_space=pltpu.HBM)] * len(args),
        out_specs=pl.BlockSpec(memory_space=pltpu.HBM),
        out_shape=jax.ShapeDtypeStruct((S, M), A_x.dtype),
        scratch_shapes=scratch,
        compiler_params=pltpu.CompilerParams(vmem_limit_bytes=120 * 1024 * 1024),
        name="adaln_cla_mod",
    )(*args)
    return out.reshape(B, S, M)
```

```python
import functools
import math

import jax
import jax.numpy as jnp
from jax import lax
import jax.experimental.pallas as pl
import jax.experimental.pallas.tpu as pltpu

F32 = jnp.float32
BF16 = jnp.bfloat16
U32 = jnp.uint32
I32 = jnp.int32

_NT = (((1,), (1,)), ((), ()))
_EPS = 1e-5
_TOPC = 8
_HG = 8
_KVR = 256
_LNR = 16
_RGR = 32
_QC = 256
_BQ = 128
_PAIRS = 1
_FQ = 256
_OH = 8
_TINY = 2.0 ** -60
_V_MAX = 2.0 ** 30
_CKV_ROWS = (256, 768, 1024)
_PROJ_ROWS = (128,) * 15 + (96, 32)
_OUT_ROWS = (1536, 512)


def _rnd(v):
    return v.astype(BF16).astype(F32)


def _adaln(x, shift, scale):
    mean = jnp.mean(x, axis=1, keepdims=True)
    d = x - mean
    var = _rnd(jnp.mean(d * d, axis=1, keepdims=True))
    den = _rnd(jnp.sqrt(_rnd(var + _rnd(jnp.full((1, 1), _EPS, F32)))))
    n = _rnd(_rnd(x - _rnd(mean)) / den)
    return _rnd(_rnd(n * _rnd(1.0 + scale)) + shift)


def _pack(v):
    return pltpu.bitcast(v.astype(BF16), U32)


def _unpack(v):
    return pltpu.bitcast(v, BF16)


def _after(words, anchor):
    zero = jnp.where(anchor * anchor < 0.0, jnp.uint32(1), jnp.uint32(0))
    return words | jnp.tile(zero, (words.shape[0] // 8, words.shape[1] // 128))


def _fold8(op, acc, v):
    for t in range(0, v.shape[0], 8):
        acc = op(acc, v[t:t + 8, :])
    return acc


def _spans(sizes):
    out, start = [], 0
    for n in sizes:
        out.append((start, n))
        start += n
    return out


def _kernel(x_hbm, ckv_hbm, wq_hbm, wuk_hbm, wuv_hbm, wo_hbm, wmod_hbm, wg_hbm,
            wu_hbm, wd_hbm, wr_hbm, c_hbm, out_hbm,
            k_v, v_v, ctx_v, h_v, wq2_v, wkv_v, x1_v, h2_v, out_v, tmp_v, col_v, wgu_v,
            x_v, ckv_v, wq_v, wuk_v, wuv_v, wo_v, wmod_v, wg_v, wu_v, wd_v, wr_v, c_v,
            mod_v, in_sems, out_sems, fix_sems):
    (S, M), Dc, (H, _, D), F = x_v.shape, ckv_v.shape[1], k_v.shape, wd_v.shape[0]
    ng = H // _HG

    started = []

    def fetch(src, dst):
        started.append(pltpu.make_async_copy(src, dst, in_sems.at[len(started)]))
        started[-1].start()
        return started[-1]

    def fetch_group(src, dst, g):
        return fetch(src.at[:, pl.ds(g * _HG, _HG), :], dst.at[g])

    def wait(copies):
        for cp in copies:
            cp.wait()

    first_weights = fetch_group(wuk_hbm, wuk_v, 0)
    ckv_copies = {a: fetch(ckv_hbm.at[pl.ds(a, n), :], ckv_v.at[pl.ds(a, n), :])
                  for a, n in _spans(_CKV_ROWS)}
    arrivals = {
        0: [fetch_group(wuv_hbm, wuv_v, 0)],
        1: [fetch_group(wuk_hbm, wuk_v, 1), fetch_group(wuv_hbm, wuv_v, 1),
            fetch(c_hbm, c_v), fetch(wmod_hbm, wmod_v)],
        3: [fetch(x_hbm, x_v)]
           + [fetch_group(src, dst, g) for g in range(2, ng)
              for src, dst in ((wuk_hbm, wuk_v), (wuv_hbm, wuv_v))]
           + [fetch_group(wq_hbm, wq_v, g) for g in range(ng)],
    }
    tail_weights = [fetch(wo_hbm, wo_v), fetch(wr_hbm, wr_v), fetch(wg_hbm, wg_v),
                    fetch(wu_hbm, wu_v), fetch(wd_hbm, wd_v)]

    def regroup(src, g, dst, pair0, a, anchor):
        n = _RGR
        tmp_v[...] = _after(pltpu.bitcast(src[g, a:a + n].reshape(n * _HG, D), U32), anchor)
        for e in range(_HG // 2):
            w = tmp_v[pl.ds(e, n, stride=_HG // 2), :]
            dst[pair0 + e, a // 2:(a + n) // 2, 0:D] = _pack(pltpu.bitcast(w << 16, F32))
            dst[pair0 + e, a // 2:(a + n) // 2, D:2 * D] = _pack(
                pltpu.bitcast(w & jnp.uint32(0xFFFF0000), F32))

    def silu_column(anchor):
        del anchor
        cf = c_v[...].astype(F32)
        col_v[...] = jnp.broadcast_to(_rnd(cf * jax.nn.sigmoid(cf)), (128, M)).T

    def modulation(t, anchor):
        w = _unpack(_after(pltpu.bitcast(wmod_v[:, t:t + 128], U32), anchor)).astype(F32)
        mod_v[t // M:t // M + 1, t % M:t % M + 128] = _rnd(
            jnp.sum(w * col_v[...], axis=0, keepdims=True))

    def x_rows(a, anchor):
        return _unpack(_after(pltpu.bitcast(x_v[a:a + _LNR, :], U32), anchor)).astype(F32)

    def first_adaln(a, anchor):
        h = _adaln(x_rows(a, anchor), mod_v[0:1, :], mod_v[1:2, :])
        h_v[a // 2:(a + _LNR) // 2, :] = _pack(h)

    released = {
        1: [silu_column] + [job for t in range(0, 6 * M, 128)
                            for job in (functools.partial(modulation, t), None, None)],
        3: [functools.partial(first_adaln, a) for a in range(0, S, _LNR)]
           + [functools.partial(regroup, wq_v, g, wq2_v, g * (_HG // 2), a)
              for g in range(ng) for a in range(0, M, _RGR)],
    }
    stages = [(src, g, o_v) for g in range(ng) for src, o_v in ((wuk_v, k_v), (wuv_v, v_v))]
    jobs = []
    first_weights.wait()
    for t, (src, g, o_v) in enumerate(stages):
        for r0 in range(0, S, _KVR):
            if t == 0 and r0 in ckv_copies:
                ckv_copies[r0].wait()
                if r0 == 0:
                    w0 = src[g].reshape(Dc, _HG * D)
            if r0 == S // 2 and t + 1 < len(stages):
                wait(arrivals.get(t, []))
                jobs = [functools.partial(regroup, *stages[t + 1][:2], wkv_v,
                                          (t + 1) % 2 * (_HG // 2), a)
                        for a in range(0, Dc, _RGR)] + jobs + released.get(t, [])
            for e0 in range(0, _HG, 4):
                if t == 0:
                    w = w0[:, e0 * D:(e0 + 4) * D]
                else:
                    w = jnp.concatenate([_unpack(wkv_v[t % 2 * (_HG // 2) + e0 // 2 + e])
                                         for e in range(2)], axis=1)
                r = jnp.dot(ckv_v[r0:r0 + _KVR, :], w, preferred_element_type=F32)
                for e in range(4):
                    head = r[:, e * D:(e + 1) * D]
                    o_v[g * _HG + e0 + e, r0 // 2:(r0 + _KVR) // 2, :] = _pack(head)
                    job = jobs.pop(0) if jobs else None
                    if job is not None:
                        job(head[0:8, :])
    assert not jobs

    qscale = float(D ** -0.5 * math.log2(math.e))
    neg = float(-1e9 * math.log2(math.e))
    nb = S // _BQ
    hb = _BQ // 2

    def attention(step, seen):
        causal = (lax.broadcasted_iota(I32, (_BQ, _BQ), 1)
                  <= lax.broadcasted_iota(I32, (_BQ, _BQ), 0))
        qs = {}

        def q_project(pair, c):
            hc = _unpack(h_v[c * _QC // 2:(c + 1) * _QC // 2, :])
            q = jnp.dot(hc, _unpack(wq2_v[_PAIRS * step + pair]),
                        preferred_element_type=F32) * qscale
            for e in range(2):
                for t in range(_QC // _BQ):
                    qs[2 * pair + e, c * _QC // _BQ + t] = (
                        q[t * _BQ:(t + 1) * _BQ, e * D:(e + 1) * D].astype(BF16))

        def scores(e, i):
            n = i * _BQ
            k = _unpack(k_v[2 * _PAIRS * step + e, 0:(i + 1) * hb, :])
            s = lax.dot_general(qs.pop((e, i)), k, _NT, preferred_element_type=F32)
            sd = jnp.where(causal, s[:, n:], neg)
            return jnp.concatenate([s[:, :n], sd], axis=1) if n else sd

        def context(e, i, s, seen):
            p = jnp.exp2(s)
            l = jnp.sum(p, axis=1, keepdims=True)
            v = _unpack(v_v[2 * _PAIRS * step + e, 0:(i + 1) * hb, :])
            o = jnp.dot(p.astype(BF16), v, preferred_element_type=F32)
            ctx_v[2 * _PAIRS * step + e, i * hb:(i + 1) * hb, :] = _pack(o * (1.0 / l))
            mag = jnp.maximum(jnp.abs(o), l * _TINY)
            return (_fold8(jnp.minimum, seen[0], mag), _fold8(jnp.maximum, seen[1], mag),
                    _fold8(jnp.minimum, seen[2], jnp.broadcast_to(l, mag.shape)),
                    _fold8(jnp.maximum, seen[3], jnp.abs(v[i * _BQ:, :].astype(F32))))

        seq = [(2 * pair + e, i) for pair in range(_PAIRS) for t in range(nb // 2)
               for e in range(2) for i in (t, nb - 1 - t)]
        projected, pending = [], None
        for t, (e, i) in enumerate(seq):
            for e2, i2 in seq[t:t + 3]:
                if (e2 // 2, i2 * _BQ // _QC) not in projected:
                    projected.append((e2 // 2, i2 * _BQ // _QC))
                    q_project(*projected[-1])
            s = scores(e, i)
            if pending is not None:
                seen = context(*pending, seen)
            pending = (e, i, s)
        return context(*pending, seen)

    ones = jnp.ones((8, D), F32)
    mag_lo, mag_hi, l_lo, v_hi = lax.fori_loop(0, H // (2 * _PAIRS), attention, (ones,) * 4)
    safe = ((mag_hi <= 1.0 / _TINY) & (l_lo >= _TINY) & (mag_lo >= _TINY)
            & (v_hi <= _V_MAX))

    @pl.when(jnp.max(jnp.where(safe, 0.0, 1.0)) > 0.0)
    def _true_max_attention():
        def body(t, carry):
            j, b = t // (S // _FQ), t % (S // _FQ)
            rows = pl.ds(pl.multiple_of(b * (_FQ // 2), _FQ // 2), _FQ // 2)
            q = jnp.dot(_unpack(h_v[rows, :]), _unpack(wq2_v[j]),
                        preferred_element_type=F32) * qscale
            causal = (lax.broadcasted_iota(I32, (_FQ, S), 1)
                      <= lax.broadcasted_iota(I32, (_FQ, S), 0) + b * _FQ)
            for e in range(2):
                s = lax.dot_general(q[:, e * D:(e + 1) * D].astype(BF16),
                                    _unpack(k_v[2 * j + e]), _NT, preferred_element_type=F32)
                s = jnp.where(causal, s, neg)
                p = jnp.exp2(s - jnp.max(s, axis=1, keepdims=True))
                p = p * (1.0 / jnp.sum(p, axis=1, keepdims=True))
                ctx_v[2 * j + e, rows, :] = _pack(jnp.dot(
                    p.astype(BF16), _unpack(v_v[2 * j + e]), preferred_element_type=F32))
            return carry

        lax.fori_loop(0, (H // 2) * (S // _FQ), body, 0)

    wait(tail_weights)
    wr = wr_v[...].astype(F32).reshape(1, M)
    lane = lax.broadcasted_iota(I32, (8, 128), 1)
    tiles = [jnp.zeros((8, 128), F32) for _ in range(S // 1024)]

    def second_adaln(a, att, anchor):
        att = pltpu.bitcast(_after(pltpu.bitcast(att, U32), anchor), F32)
        x1 = _rnd(x_rows(a, anchor) + _rnd(mod_v[2:3, :] * _rnd(att)))
        h2 = _adaln(x1, mod_v[3:4, :], mod_v[4:5, :])
        x1_v[a:a + _LNR, :] = x1
        h2_v[a:a + _LNR, :] = h2
        out_v[a:a + _LNR, :] = (x1 + _rnd(mod_v[5:6, :] * (h2 + h2 * 0.0))).astype(BF16)
        r = jnp.sum(h2 * wr, axis=1, keepdims=True)
        for u in range(0, _LNR, 8):
            t, ln = divmod((a + u) // 8, 128)
            tiles[t] = jnp.where(lane == ln, r[u:u + 8, :], tiles[t])

    def untranspose(src, which, f0, m0, anchor):
        n = min(128, F - f0)
        w = _unpack(_after(pltpu.bitcast(src[f0:f0 + n, m0:m0 + 128], U32), anchor))
        wgu_v[which, m0 // 2:(m0 + 128) // 2, f0:f0 + n] = _pack(w.astype(F32).T)

    spare = [functools.partial(untranspose, src, which, f0, m0)
             for which, src in enumerate((wg_v, wu_v))
             for f0 in range(0, F, 128) for m0 in range(0, M, 128)]
    out_copies = [
        pltpu.make_async_copy(out_v.at[pl.ds(a, n), :], out_hbm.at[pl.ds(a, n), :], out_sems.at[i])
        for i, (a, n) in enumerate(_spans(_OUT_ROWS))]
    for r0, n in _spans(_PROJ_ROWS):
        parts = []
        for c0 in range(0, M, 128):
            acc = None
            for h0 in range(0, H, _OH):
                ctx = jnp.concatenate([_unpack(ctx_v[h, r0 // 2:(r0 + n) // 2, :])
                                       for h in range(h0, h0 + _OH)], axis=1)
                part = jnp.dot(ctx, wo_v[h0 * D:(h0 + _OH) * D, c0:c0 + 128],
                               preferred_element_type=F32)
                acc = part if acc is None else acc + part
                odd = h0 // _OH % 2
                queue = spare if spare and (odd or not jobs) else jobs
                if queue:
                    queue.pop(0)(part[0:8, :])
            parts.append(acc)
        assert not jobs
        if r0 == _OUT_ROWS[0]:
            out_copies[0].start()
        att = jnp.concatenate(parts, axis=1)
        jobs = [functools.partial(second_adaln, r0 + t, att[t:t + _LNR, :])
                for t in range(0, n, _LNR)]
    assert not spare
    for job in jobs:
        job(att[0:8, 0:128])
    out_copies[1].start()

    r = _rnd(jnp.concatenate(tiles, axis=0))
    sub = lax.broadcasted_iota(I32, r.shape, 0)
    tok = (sub // 8) * 1024 + lax.broadcasted_iota(I32, r.shape, 1) * 8 + sub % 8
    bits = pltpu.bitcast(jnp.where(r == 0.0, 0.0, r), I32) >> 16
    order = jnp.where(bits < 0, -(bits & 0x7FFF), bits) + 0x8000
    order = jnp.where(r != r, 0, order)
    key = pltpu.bitcast((order * S + (S - 1 - tok)) + 0x20000000, F32)
    idx = []
    for _ in range(_TOPC):
        top = jnp.max(jnp.max(key, axis=0, keepdims=True), axis=1, keepdims=True)
        idx.append((S - 1) - (pltpu.bitcast(top, I32)[0, 0] & (S - 1)))
        key = jnp.where(key == top, 0.0, key)

    hs = jnp.concatenate([h2_v[pl.ds(i, 1), :] for i in idx], axis=0)
    xs = jnp.concatenate([x1_v[pl.ds(i, 1), :] for i in idx], axis=0)
    hs16 = jnp.concatenate([hs, hs], axis=0).astype(BF16)
    g = _rnd(jnp.dot(hs16, _unpack(wgu_v[0]), preferred_element_type=F32))
    u = _rnd(jnp.dot(hs16, _unpack(wgu_v[1]), preferred_element_type=F32))
    act = (_rnd(g * jax.nn.sigmoid(g)) * u).astype(BF16)
    y = _rnd(jnp.dot(act, wd_v[...], preferred_element_type=F32))[0:_TOPC, :]
    rs = _rnd(jnp.sum(hs * wr, axis=1, keepdims=True))
    y = _rnd(y * _rnd(jax.nn.sigmoid(rs)))
    new = xs + _rnd(mod_v[5:6, :] * _rnd(hs + _rnd(hs * 0.0 + y)))

    wait(out_copies)
    sub16 = lax.broadcasted_iota(I32, (16, M), 0)
    groups = [pl.ds(pl.multiple_of((i // 16) * 16, 16), 16) for i in idx]
    for n, i in enumerate(idx):
        old = out_v[groups[n], :].astype(F32)
        out_v[groups[n], :] = jnp.where(sub16 == i % 16, new[n:n + 1, :], old).astype(BF16)
    fixes = []
    for n, i in enumerate(idx):
        first = True
        for prev in idx[:n]:
            first = (prev // 16 != i // 16) & first
        fixes.append((first, pltpu.make_async_copy(
            out_v.at[groups[n], :], out_hbm.at[groups[n], :], fix_sems.at[n])))
    for first, cp in fixes:
        pl.when(first)(cp.start)
    for first, cp in fixes:
        pl.when(first)(cp.wait)


@jax.jit
def pallas_adaLN_cond__compressed_kv_cla__moe_arch_mod__prompt_kernel(
    A_x: jax.Array,
    A_c_kv: jax.Array,
    A_w_q: jax.Array,
    A_w_uk: jax.Array,
    A_w_uv: jax.Array,
    A_w_o: jax.Array,
    B_x: jax.Array,
    B_w_r: jax.Array,
    B_w_gate: jax.Array,
    B_w_up: jax.Array,
    B_w_down: jax.Array,
    c: jax.Array,
    w_mod: jax.Array,
):
    del B_x
    B, S, M = A_x.shape
    Dc = A_c_kv.shape[2]
    _, H, D = A_w_q.shape
    F = B_w_down.shape[0]
    assert B == 1 and A_c_kv.shape[1] == S
    assert S == sum(_CKV_ROWS) == sum(_PROJ_ROWS) == sum(_OUT_ROWS)

    args = (
        A_x.reshape(S, M), A_c_kv.reshape(S, Dc), A_w_q, A_w_uk, A_w_uv,
        A_w_o.reshape(H * D, M), w_mod, B_w_gate.T, B_w_up.T, B_w_down, B_w_r, c,
    )
    ng = H // _HG
    scratch = [
        pltpu.VMEM((H, S // 2, D), U32),
        pltpu.VMEM((H, S // 2, D), U32),
        pltpu.VMEM((H, S // 2, D), U32),
        pltpu.VMEM((S // 2, M), U32),
        pltpu.VMEM((H // 2, M // 2, 2 * D), U32),
        pltpu.VMEM((_HG, Dc // 2, 2 * D), U32),
        pltpu.VMEM((S, M), F32),
        pltpu.VMEM((S, M), F32),
        pltpu.VMEM((S, M), BF16),
        pltpu.VMEM((_RGR * _HG // 2, D), U32),
        pltpu.VMEM((M, 128), F32),
        pltpu.VMEM((2, M // 2, F), U32),
    ] + [
        pltpu.VMEM((ng, a.shape[0], _HG, D) if a.ndim == 3 else a.shape, a.dtype)
        for a in args
    ] + [
        pltpu.VMEM((8, M), F32),
        pltpu.SemaphoreType.DMA((3 * ng + len(_CKV_ROWS) + 8,)),
        pltpu.SemaphoreType.DMA((len(_OUT_ROWS),)),
        pltpu.SemaphoreType.DMA((_TOPC,)),
    ]

    out = pl.pallas_call(
        _kernel,
        in_specs=[pl.BlockSpec(memory_space=pltpu.HBM)] * len(args),
        out_specs=pl.BlockSpec(memory_space=pltpu.HBM),
        out_shape=jax.ShapeDtypeStruct((S, M), A_x.dtype),
        scratch_shapes=scratch,
        compiler_params=pltpu.CompilerParams(vmem_limit_bytes=120 * 1024 * 1024),
        name="adaln_cla_mod",
    )(*args)
    return out.reshape(B, S, M)
```

```python
import functools
import math

import jax
import jax.numpy as jnp
from jax import lax
import jax.experimental.pallas as pl
import jax.experimental.pallas.tpu as pltpu

F32 = jnp.float32
BF16 = jnp.bfloat16
U32 = jnp.uint32
I32 = jnp.int32

_NT = (((1,), (1,)), ((), ()))
_EPS = 1e-5
_TOPC = 8
_HG = 8
_KVR = 256
_LNR = 16
_RGR = 32
_MDR = 320
_QC = 256
_BQ = 128
_PAIRS = 1
_FQ = 256
_OH = 8
_TINY = 2.0 ** -60
_V_MAX = 2.0 ** 30
_CKV_ROWS = (256, 768, 1024)
_PROJ_ROWS = (128,) * 15 + (96, 32)
_OUT_ROWS = (1536, 512)


def _rnd(v):
    return v.astype(BF16).astype(F32)


def _adaln(x, shift, scale):
    mean = jnp.mean(x, axis=1, keepdims=True)
    d = x - mean
    var = _rnd(jnp.mean(d * d, axis=1, keepdims=True))
    den = _rnd(jnp.sqrt(_rnd(var + _rnd(jnp.full((1, 1), _EPS, F32)))))
    n = _rnd(_rnd(x - _rnd(mean)) / den)
    return _rnd(_rnd(n * _rnd(1.0 + scale)) + shift)


def _sigmoid(x):
    return _rnd(1.0 / _rnd(1.0 + _rnd(jnp.exp(-x))))


def _pack(v):
    return pltpu.bitcast(v.astype(BF16), U32)


def _unpack(v):
    return pltpu.bitcast(v, BF16)


def _after(words, anchor):
    zero = jnp.where(anchor * anchor < 0.0, jnp.uint32(1), jnp.uint32(0))
    return words | jnp.tile(zero, (words.shape[0] // 8, words.shape[1] // 128))


def _fold8(op, acc, v):
    for t in range(0, v.shape[0], 8):
        acc = op(acc, v[t:t + 8, :])
    return acc


def _spans(sizes):
    out, start = [], 0
    for n in sizes:
        out.append((start, n))
        start += n
    return out


def _kernel(x_hbm, ckv_hbm, wq_hbm, wuk_hbm, wuv_hbm, wo_hbm, wmod_hbm, wg_hbm,
            wu_hbm, wd_hbm, wr_hbm, c_hbm, out_hbm,
            k_v, v_v, ctx_v, h_v, wq2_v, wkv_v, x1_v, h2_v, out_v, tmp_v, col_v, wgu_v,
            x_v, ckv_v, wq_v, wuk_v, wuv_v, wo_v, wmod_v, wg_v, wu_v, wd_v, wr_v, c_v,
            mod_v, in_sems, out_sems, fix_sems):
    (S, M), Dc, (H, _, D), F = x_v.shape, ckv_v.shape[1], k_v.shape, wd_v.shape[0]
    ng = H // _HG

    started = []

    def fetch(src, dst):
        started.append(pltpu.make_async_copy(src, dst, in_sems.at[len(started)]))
        started[-1].start()
        return started[-1]

    def fetch_group(src, dst, g):
        return fetch(src.at[:, pl.ds(g * _HG, _HG), :], dst.at[g])

    def wait(copies):
        for cp in copies:
            cp.wait()

    first_weights = fetch_group(wuk_hbm, wuk_v, 0)
    ckv_copies = {a: fetch(ckv_hbm.at[pl.ds(a, n), :], ckv_v.at[pl.ds(a, n), :])
                  for a, n in _spans(_CKV_ROWS)}
    arrivals = {
        0: [fetch_group(wuv_hbm, wuv_v, 0)],
        1: [fetch_group(wuk_hbm, wuk_v, 1), fetch_group(wuv_hbm, wuv_v, 1),
            fetch(c_hbm, c_v), fetch(wmod_hbm, wmod_v)],
        3: [fetch(x_hbm, x_v)]
           + [fetch_group(src, dst, g) for g in range(2, ng)
              for src, dst in ((wuk_hbm, wuk_v), (wuv_hbm, wuv_v))]
           + [fetch_group(wq_hbm, wq_v, g) for g in range(ng)],
    }
    tail_weights = [fetch(wo_hbm, wo_v), fetch(wr_hbm, wr_v), fetch(wg_hbm, wg_v),
                    fetch(wu_hbm, wu_v), fetch(wd_hbm, wd_v)]

    def regroup(src, g, dst, pair0, a, anchor):
        n = _RGR
        tmp_v[...] = _after(pltpu.bitcast(src[g, a:a + n].reshape(n * _HG, D), U32), anchor)
        for e in range(_HG // 2):
            w = tmp_v[pl.ds(e, n, stride=_HG // 2), :]
            dst[pair0 + e, a // 2:(a + n) // 2, 0:D] = _pack(pltpu.bitcast(w << 16, F32))
            dst[pair0 + e, a // 2:(a + n) // 2, D:2 * D] = _pack(
                pltpu.bitcast(w & jnp.uint32(0xFFFF0000), F32))

    def silu_column(anchor):
        del anchor
        cf = c_v[...].astype(F32)
        col_v[...] = jnp.broadcast_to(_rnd(cf * _sigmoid(cf)), (128, M)).T

    partial_mod = {}

    def modulation(t, a, anchor):
        w = pltpu.bitcast(wmod_v[a:a + _MDR, t:t + 128], U32)
        prod = _unpack(_after(w, anchor)).astype(F32) * col_v[a:a + _MDR, :]
        partial_mod[t] = _fold8(jnp.add, partial_mod.get(t, 0.0), prod)
        if a + _MDR == M:
            mod_v[t // M:t // M + 1, t % M:t % M + 128] = _rnd(
                jnp.sum(partial_mod.pop(t), axis=0, keepdims=True))

    def x_rows(a, anchor):
        return _unpack(_after(pltpu.bitcast(x_v[a:a + _LNR, :], U32), anchor)).astype(F32)

    def first_adaln(a, anchor):
        h = _adaln(x_rows(a, anchor), mod_v[0:1, :], mod_v[1:2, :])
        h_v[a // 2:(a + _LNR) // 2, :] = _pack(h)

    released = {
        1: [silu_column] + [functools.partial(modulation, t, a)
                            for t in range(0, 6 * M, 128) for a in range(0, M, _MDR)],
        3: [functools.partial(first_adaln, a) for a in range(0, S, _LNR)]
           + [functools.partial(regroup, wq_v, g, wq2_v, g * (_HG // 2), a)
              for g in range(ng) for a in range(0, M, _RGR)],
    }
    stages = [(src, g, o_v) for g in range(ng) for src, o_v in ((wuk_v, k_v), (wuv_v, v_v))]
    jobs = []
    first_weights.wait()
    for t, (src, g, o_v) in enumerate(stages):
        for r0 in range(0, S, _KVR):
            if t == 0 and r0 in ckv_copies:
                ckv_copies[r0].wait()
                if r0 == 0:
                    w0 = src[g].reshape(Dc, _HG * D)
            if r0 == S // 2 and t + 1 < len(stages):
                wait(arrivals.get(t, []))
                jobs = [functools.partial(regroup, *stages[t + 1][:2], wkv_v,
                                          (t + 1) % 2 * (_HG // 2), a)
                        for a in range(0, Dc, _RGR)] + jobs + released.get(t, [])
            for e0 in range(0, _HG, 4):
                if t == 0:
                    w = w0[:, e0 * D:(e0 + 4) * D]
                else:
                    w = jnp.concatenate([_unpack(wkv_v[t % 2 * (_HG // 2) + e0 // 2 + e])
                                         for e in range(2)], axis=1)
                r = jnp.dot(ckv_v[r0:r0 + _KVR, :], w, preferred_element_type=F32)
                for e in range(4):
                    head = r[:, e * D:(e + 1) * D]
                    o_v[g * _HG + e0 + e, r0 // 2:(r0 + _KVR) // 2, :] = _pack(head)
                    if jobs:
                        jobs.pop(0)(head[0:8, :])
    assert not jobs

    qscale = float(D ** -0.5 * math.log2(math.e))
    neg = float(-1e9 * math.log2(math.e))
    nb = S // _BQ
    hb = _BQ // 2

    def attention(step, seen):
        causal = (lax.broadcasted_iota(I32, (_BQ, _BQ), 1)
                  <= lax.broadcasted_iota(I32, (_BQ, _BQ), 0))
        qs = {}

        def q_project(pair, c):
            hc = _unpack(h_v[c * _QC // 2:(c + 1) * _QC // 2, :])
            q = jnp.dot(hc, _unpack(wq2_v[_PAIRS * step + pair]),
                        preferred_element_type=F32) * qscale
            for e in range(2):
                for t in range(_QC // _BQ):
                    qs[2 * pair + e, c * _QC // _BQ + t] = (
                        q[t * _BQ:(t + 1) * _BQ, e * D:(e + 1) * D].astype(BF16))

        def scores(e, i):
            n = i * _BQ
            k = _unpack(k_v[2 * _PAIRS * step + e, 0:(i + 1) * hb, :])
            s = lax.dot_general(qs.pop((e, i)), k, _NT, preferred_element_type=F32)
            sd = jnp.where(causal, s[:, n:], neg)
            return jnp.concatenate([s[:, :n], sd], axis=1) if n else sd

        def context(e, i, s, seen):
            p = jnp.exp2(s)
            l = jnp.sum(p, axis=1, keepdims=True)
            v = _unpack(v_v[2 * _PAIRS * step + e, 0:(i + 1) * hb, :])
            o = jnp.dot(p.astype(BF16), v, preferred_element_type=F32)
            ctx_v[2 * _PAIRS * step + e, i * hb:(i + 1) * hb, :] = _pack(o * (1.0 / l))
            mag = jnp.maximum(jnp.abs(o), l * _TINY)
            return (_fold8(jnp.minimum, seen[0], mag), _fold8(jnp.maximum, seen[1], mag),
                    _fold8(jnp.minimum, seen[2], jnp.broadcast_to(l, mag.shape)),
                    _fold8(jnp.maximum, seen[3], jnp.abs(v[i * _BQ:, :].astype(F32))))

        seq = [(2 * pair + e, i) for pair in range(_PAIRS) for t in range(nb // 2)
               for e in range(2) for i in (t, nb - 1 - t)]
        projected, pending = [], None
        for t, (e, i) in enumerate(seq):
            for e2, i2 in seq[t:t + 3]:
                if (e2 // 2, i2 * _BQ // _QC) not in projected:
                    projected.append((e2 // 2, i2 * _BQ // _QC))
                    q_project(*projected[-1])
            s = scores(e, i)
            if pending is not None:
                seen = context(*pending, seen)
            pending = (e, i, s)
        return context(*pending, seen)

    ones = jnp.ones((8, D), F32)
    mag_lo, mag_hi, l_lo, v_hi = lax.fori_loop(0, H // (2 * _PAIRS), attention, (ones,) * 4)
    safe = ((mag_hi <= 1.0 / _TINY) & (l_lo >= _TINY) & (mag_lo >= _TINY)
            & (v_hi <= _V_MAX))

    @pl.when(jnp.max(jnp.where(safe, 0.0, 1.0)) > 0.0)
    def _true_max_attention():
        def body(t, carry):
            j, b = t // (S // _FQ), t % (S // _FQ)
            rows = pl.ds(pl.multiple_of(b * (_FQ // 2), _FQ // 2), _FQ // 2)
            q = jnp.dot(_unpack(h_v[rows, :]), _unpack(wq2_v[j]),
                        preferred_element_type=F32) * qscale
            causal = (lax.broadcasted_iota(I32, (_FQ, S), 1)
                      <= lax.broadcasted_iota(I32, (_FQ, S), 0) + b * _FQ)
            for e in range(2):
                s = lax.dot_general(q[:, e * D:(e + 1) * D].astype(BF16),
                                    _unpack(k_v[2 * j + e]), _NT, preferred_element_type=F32)
                s = jnp.where(causal, s, neg)
                p = jnp.exp2(s - jnp.max(s, axis=1, keepdims=True))
                p = p * (1.0 / jnp.sum(p, axis=1, keepdims=True))
                ctx_v[2 * j + e, rows, :] = _pack(jnp.dot(
                    p.astype(BF16), _unpack(v_v[2 * j + e]), preferred_element_type=F32))
            return carry

        lax.fori_loop(0, (H // 2) * (S // _FQ), body, 0)

    wait(tail_weights)
    wr = wr_v[...].astype(F32).reshape(1, M)
    lane = lax.broadcasted_iota(I32, (8, 128), 1)
    tiles = [jnp.zeros((8, 128), F32) for _ in range(S // 1024)]

    def second_adaln(a, att, anchor):
        att = pltpu.bitcast(_after(pltpu.bitcast(att, U32), anchor), F32)
        x1 = _rnd(x_rows(a, anchor) + _rnd(mod_v[2:3, :] * _rnd(att)))
        h2 = _adaln(x1, mod_v[3:4, :], mod_v[4:5, :])
        x1_v[a:a + _LNR, :] = x1
        h2_v[a:a + _LNR, :] = h2
        out_v[a:a + _LNR, :] = (x1 + _rnd(mod_v[5:6, :] * (h2 + h2 * 0.0))).astype(BF16)
        r = jnp.sum(h2 * wr, axis=1, keepdims=True)
        for u in range(0, _LNR, 8):
            t, ln = divmod((a + u) // 8, 128)
            tiles[t] = jnp.where(lane == ln, r[u:u + 8, :], tiles[t])

    def untranspose(src, which, f0, m0, anchor):
        n = min(128, F - f0)
        w = _unpack(_after(pltpu.bitcast(src[f0:f0 + n, m0:m0 + 128], U32), anchor))
        wgu_v[which, m0 // 2:(m0 + 128) // 2, f0:f0 + n] = _pack(w.T)

    spare = [functools.partial(untranspose, src, which, f0, m0)
             for which, src in enumerate((wg_v, wu_v))
             for f0 in range(0, F, 128) for m0 in range(0, M, 128)]
    out_copies = [
        pltpu.make_async_copy(out_v.at[pl.ds(a, n), :], out_hbm.at[pl.ds(a, n), :], out_sems.at[i])
        for i, (a, n) in enumerate(_spans(_OUT_ROWS))]
    for r0, n in _spans(_PROJ_ROWS):
        parts = []
        for c0 in range(0, M, 128):
            acc = None
            for h0 in range(0, H, _OH):
                ctx = jnp.concatenate([_unpack(ctx_v[h, r0 // 2:(r0 + n) // 2, :])
                                       for h in range(h0, h0 + _OH)], axis=1)
                part = jnp.dot(ctx, wo_v[h0 * D:(h0 + _OH) * D, c0:c0 + 128],
                               preferred_element_type=F32)
                acc = part if acc is None else acc + part
                odd = h0 // _OH % 2
                queue = spare if spare and (odd or not jobs) else jobs
                if queue:
                    queue.pop(0)(part[0:8, :])
            parts.append(acc)
        assert not jobs
        if r0 == _OUT_ROWS[0]:
            out_copies[0].start()
        att = jnp.concatenate(parts, axis=1)
        jobs = [functools.partial(second_adaln, r0 + t, att[t:t + _LNR, :])
                for t in range(0, n, _LNR)]
    assert not spare
    for job in jobs:
        job(att[0:8, 0:128])
    out_copies[1].start()

    r = _rnd(jnp.concatenate(tiles, axis=0))
    sub = lax.broadcasted_iota(I32, r.shape, 0)
    tok = (sub // 8) * 1024 + lax.broadcasted_iota(I32, r.shape, 1) * 8 + sub % 8
    bits = pltpu.bitcast(jnp.where(r == 0.0, 0.0, r), I32) >> 16
    order = jnp.where(bits < 0, -(bits & 0x7FFF), bits) + 0x8000
    order = jnp.where(r != r, 0, order)
    key = pltpu.bitcast((order * S + (S - 1 - tok)) + 0x20000000, F32)
    idx = []
    for _ in range(_TOPC):
        top = jnp.max(jnp.max(key, axis=0, keepdims=True), axis=1, keepdims=True)
        idx.append((S - 1) - (pltpu.bitcast(top, I32)[0, 0] & (S - 1)))
        key = jnp.where(key == top, 0.0, key)

    hs = jnp.concatenate([h2_v[pl.ds(i, 1), :] for i in idx], axis=0)
    xs = jnp.concatenate([x1_v[pl.ds(i, 1), :] for i in idx], axis=0)
    hs16 = jnp.concatenate([hs, hs], axis=0).astype(BF16)
    g = _rnd(jnp.dot(hs16, _unpack(wgu_v[0]), preferred_element_type=F32))
    u = _rnd(jnp.dot(hs16, _unpack(wgu_v[1]), preferred_element_type=F32))
    act = (_rnd(g * _sigmoid(g)) * u).astype(BF16)
    y = _rnd(jnp.dot(act, wd_v[...], preferred_element_type=F32))[0:_TOPC, :]
    rs = _rnd(jnp.sum(hs * wr, axis=1, keepdims=True))
    y = _rnd(y * _sigmoid(rs))
    new = xs + _rnd(mod_v[5:6, :] * _rnd(hs + _rnd(hs * 0.0 + y)))

    wait(out_copies)
    sub16 = lax.broadcasted_iota(I32, (16, M), 0)
    groups = [pl.ds(pl.multiple_of((i // 16) * 16, 16), 16) for i in idx]
    for n, i in enumerate(idx):
        old = out_v[groups[n], :].astype(F32)
        out_v[groups[n], :] = jnp.where(sub16 == i % 16, new[n:n + 1, :], old).astype(BF16)
    fixes = []
    for n, i in enumerate(idx):
        first = True
        for prev in idx[:n]:
            first = (prev // 16 != i // 16) & first
        fixes.append((first, pltpu.make_async_copy(
            out_v.at[groups[n], :], out_hbm.at[groups[n], :], fix_sems.at[n])))
    for first, cp in fixes:
        pl.when(first)(cp.start)
    for first, cp in fixes:
        pl.when(first)(cp.wait)


@jax.jit
def pallas_adaLN_cond__compressed_kv_cla__moe_arch_mod__prompt_kernel(
    A_x: jax.Array,
    A_c_kv: jax.Array,
    A_w_q: jax.Array,
    A_w_uk: jax.Array,
    A_w_uv: jax.Array,
    A_w_o: jax.Array,
    B_x: jax.Array,
    B_w_r: jax.Array,
    B_w_gate: jax.Array,
    B_w_up: jax.Array,
    B_w_down: jax.Array,
    c: jax.Array,
    w_mod: jax.Array,
):
    del B_x
    B, S, M = A_x.shape
    Dc = A_c_kv.shape[2]
    _, H, D = A_w_q.shape
    F = B_w_down.shape[0]
    assert B == 1 and A_c_kv.shape[1] == S
    assert S == sum(_CKV_ROWS) == sum(_PROJ_ROWS) == sum(_OUT_ROWS)

    args = (
        A_x.reshape(S, M), A_c_kv.reshape(S, Dc), A_w_q, A_w_uk, A_w_uv,
        A_w_o.reshape(H * D, M), w_mod, B_w_gate.T, B_w_up.T, B_w_down, B_w_r, c,
    )
    ng = H // _HG
    scratch = [
        pltpu.VMEM((H, S // 2, D), U32),
        pltpu.VMEM((H, S // 2, D), U32),
        pltpu.VMEM((H, S // 2, D), U32),
        pltpu.VMEM((S // 2, M), U32),
        pltpu.VMEM((H // 2, M // 2, 2 * D), U32),
        pltpu.VMEM((_HG, Dc // 2, 2 * D), U32),
        pltpu.VMEM((S, M), F32),
        pltpu.VMEM((S, M), F32),
        pltpu.VMEM((S, M), BF16),
        pltpu.VMEM((_RGR * _HG // 2, D), U32),
        pltpu.VMEM((M, 128), F32),
        pltpu.VMEM((2, M // 2, F), U32),
    ] + [
        pltpu.VMEM((ng, a.shape[0], _HG, D) if a.ndim == 3 else a.shape, a.dtype)
        for a in args
    ] + [
        pltpu.VMEM((8, M), F32),
        pltpu.SemaphoreType.DMA((3 * ng + len(_CKV_ROWS) + 8,)),
        pltpu.SemaphoreType.DMA((len(_OUT_ROWS),)),
        pltpu.SemaphoreType.DMA((_TOPC,)),
    ]

    out = pl.pallas_call(
        _kernel,
        in_specs=[pl.BlockSpec(memory_space=pltpu.HBM)] * len(args),
        out_specs=pl.BlockSpec(memory_space=pltpu.HBM),
        out_shape=jax.ShapeDtypeStruct((S, M), A_x.dtype),
        scratch_shapes=scratch,
        compiler_params=pltpu.CompilerParams(vmem_limit_bytes=120 * 1024 * 1024),
        name="adaln_cla_mod",
    )(*args)
    return out.reshape(B, S, M)
```

```python
import functools
import math

import jax
import jax.numpy as jnp
from jax import lax
import jax.experimental.pallas as pl
import jax.experimental.pallas.tpu as pltpu

F32 = jnp.float32
BF16 = jnp.bfloat16
U32 = jnp.uint32
I32 = jnp.int32

_NT = (((1,), (1,)), ((), ()))
_EPS = 1e-5
_TOPC = 8
_HG = 8
_KVR = 256
_LNR = 16
_RGR = 64
_MDR = 320
_QC = 256
_BQ = 128
_FQ = 256
_OH = 8
_TINY = 2.0 ** -60
_V_MAX = 2.0 ** 30
_CKV_ROWS = (256, 768, 1024)
_PROJ_ROWS = (128,) * 15 + (96, 32)
_OUT_ROWS = (1536, 512)


def _rnd(v):
    return v.astype(BF16).astype(F32)


def _adaln(x, shift, scale):
    mean = jnp.mean(x, axis=1, keepdims=True)
    d = x - mean
    var = _rnd(jnp.mean(d * d, axis=1, keepdims=True))
    den = _rnd(jnp.sqrt(_rnd(var + _rnd(jnp.full((1, 1), _EPS, F32)))))
    n = _rnd(_rnd(x - _rnd(mean)) / den)
    return _rnd(_rnd(n * _rnd(1.0 + scale)) + shift)


def _sigmoid(x):
    return _rnd(1.0 / _rnd(1.0 + _rnd(jnp.exp(-x))))


def _pack(v):
    return pltpu.bitcast(v.astype(BF16), U32)


def _unpack(v):
    return pltpu.bitcast(v, BF16)


def _after(words, anchor):
    zero = jnp.where(anchor * anchor < 0.0, jnp.uint32(1), jnp.uint32(0))
    return words | jnp.tile(zero, (words.shape[0] // 8, words.shape[1] // 128))


def _tiles(v):
    return v.reshape(v.shape[0] // 8, 8, v.shape[1])


def _spans(sizes):
    out, start = [], 0
    for n in sizes:
        out.append((start, n))
        start += n
    return out


def _kernel(x_hbm, ckv_hbm, wq_hbm, wuk_hbm, wuv_hbm, wo_hbm, wmod_hbm, wg_hbm,
            wu_hbm, wd_hbm, wr_hbm, c_hbm, out_hbm,
            k_v, v_v, ctx_v, h_v, wq2_v, wkv_v, x1_v, h2_v, out_v, tmp_v, col_v, wgu_v,
            x_v, ckv_v, wq_v, wuk_v, wuv_v, wo_v, wmod_v, wg_v, wu_v, wd_v, wr_v, c_v,
            mod_v, in_sems, out_sems, fix_sems):
    (S, M), Dc, (H, _, D), F = x_v.shape, ckv_v.shape[1], k_v.shape, wd_v.shape[0]
    ng = H // _HG

    started = []

    def fetch(src, dst):
        started.append(pltpu.make_async_copy(src, dst, in_sems.at[len(started)]))
        started[-1].start()
        return started[-1]

    def fetch_group(src, dst, g):
        return fetch(src.at[:, pl.ds(g * _HG, _HG), :], dst.at[g])

    def wait(copies):
        for cp in copies:
            cp.wait()

    first_weights = fetch_group(wuk_hbm, wuk_v, 0)
    ckv_copies = {a: fetch(ckv_hbm.at[pl.ds(a, n), :], ckv_v.at[pl.ds(a, n), :])
                  for a, n in _spans(_CKV_ROWS)}
    arrivals = {
        0: [fetch_group(wuv_hbm, wuv_v, 0)],
        1: [fetch_group(wuk_hbm, wuk_v, 1), fetch_group(wuv_hbm, wuv_v, 1),
            fetch(c_hbm, c_v), fetch(wmod_hbm, wmod_v)],
        3: [fetch(x_hbm, x_v)]
           + [fetch_group(src, dst, g) for g in range(2, ng)
              for src, dst in ((wuk_hbm, wuk_v), (wuv_hbm, wuv_v))]
           + [fetch_group(wq_hbm, wq_v, g) for g in range(ng)],
    }
    tail_weights = [fetch(wo_hbm, wo_v), fetch(wr_hbm, wr_v), fetch(wg_hbm, wg_v),
                    fetch(wu_hbm, wu_v), fetch(wd_hbm, wd_v)]

    def regroup(src, g, dst, pair0, a, anchor):
        n = _RGR
        tmp_v[...] = _after(pltpu.bitcast(src[g, a:a + n].reshape(n * _HG, D), U32), anchor)
        for e in range(_HG // 2):
            w = tmp_v[pl.ds(e, n, stride=_HG // 2), :]
            dst[pair0 + e, a // 2:(a + n) // 2, 0:D] = _pack(pltpu.bitcast(w << 16, F32))
            dst[pair0 + e, a // 2:(a + n) // 2, D:2 * D] = _pack(
                pltpu.bitcast(w & jnp.uint32(0xFFFF0000), F32))

    def silu_column(anchor):
        del anchor
        cf = c_v[...].astype(F32)
        col_v[...] = jnp.broadcast_to(_rnd(cf * _sigmoid(cf)), (128, M)).T

    partial_mod = {}

    def modulation(t, a, anchor):
        w = pltpu.bitcast(wmod_v[a:a + _MDR, t:t + 128], U32)
        prod = _unpack(_after(w, anchor)).astype(F32) * col_v[a:a + _MDR, :]
        partial_mod[t] = partial_mod.get(t, 0.0) + jnp.sum(_tiles(prod), axis=0)
        if a + _MDR == M:
            mod_v[t // M:t // M + 1, t % M:t % M + 128] = _rnd(
                jnp.sum(partial_mod.pop(t), axis=0, keepdims=True))

    def x_rows(a, anchor):
        return _unpack(_after(pltpu.bitcast(x_v[a:a + _LNR, :], U32), anchor)).astype(F32)

    def first_adaln(a, anchor):
        h = _adaln(x_rows(a, anchor), mod_v[0:1, :], mod_v[1:2, :])
        h_v[a // 2:(a + _LNR) // 2, :] = _pack(h)

    released = {
        1: [silu_column] + [functools.partial(modulation, t, a)
                            for t in range(0, 6 * M, 128) for a in range(0, M, _MDR)],
        3: [functools.partial(first_adaln, a) for a in range(0, S, _LNR)]
           + [functools.partial(regroup, wq_v, g, wq2_v, g * (_HG // 2), a)
              for g in range(ng) for a in range(0, M, _RGR)],
    }
    stages = [(src, g, o_v) for g in range(ng) for src, o_v in ((wuk_v, k_v), (wuv_v, v_v))]
    jobs = []
    first_weights.wait()
    for t, (src, g, o_v) in enumerate(stages):
        for r0 in range(0, S, _KVR):
            if t == 0 and r0 in ckv_copies:
                ckv_copies[r0].wait()
                if r0 == 0:
                    w0 = src[g].reshape(Dc, _HG * D)
            if r0 == S // 2 and t + 1 < len(stages):
                wait(arrivals.get(t, []))
                jobs = [functools.partial(regroup, *stages[t + 1][:2], wkv_v,
                                          (t + 1) % 2 * (_HG // 2), a)
                        for a in range(0, Dc, _RGR)] + jobs + released.get(t, [])
            for e0 in range(0, _HG, 4):
                if t == 0:
                    w = w0[:, e0 * D:(e0 + 4) * D]
                else:
                    w = jnp.concatenate([_unpack(wkv_v[t % 2 * (_HG // 2) + e0 // 2 + e])
                                         for e in range(2)], axis=1)
                r = jnp.dot(ckv_v[r0:r0 + _KVR, :], w, preferred_element_type=F32)
                for e in range(4):
                    head = r[:, e * D:(e + 1) * D]
                    o_v[g * _HG + e0 + e, r0 // 2:(r0 + _KVR) // 2, :] = _pack(head)
                    if jobs:
                        jobs.pop(0)(head[0:8, :])
    assert not jobs

    qscale = float(D ** -0.5 * math.log2(math.e))
    neg = float(-1e9 * math.log2(math.e))
    nb = S // _BQ
    hb = _BQ // 2

    def attention(j, seen):
        causal = (lax.broadcasted_iota(I32, (_BQ, _BQ), 1)
                  <= lax.broadcasted_iota(I32, (_BQ, _BQ), 0))
        qs = {}

        def q_project(c):
            hc = _unpack(h_v[c * _QC // 2:(c + 1) * _QC // 2, :])
            q = jnp.dot(hc, _unpack(wq2_v[j]), preferred_element_type=F32) * qscale
            for e in range(2):
                for t in range(_QC // _BQ):
                    qs[e, c * _QC // _BQ + t] = (
                        q[t * _BQ:(t + 1) * _BQ, e * D:(e + 1) * D].astype(BF16))

        def scores(e, i):
            n = i * _BQ
            k = _unpack(k_v[2 * j + e, 0:(i + 1) * hb, :])
            s = lax.dot_general(qs.pop((e, i)), k, _NT, preferred_element_type=F32)
            sd = jnp.where(causal, s[:, n:], neg)
            return jnp.concatenate([s[:, :n], sd], axis=1) if n else sd

        def context(e, i, s, seen):
            p = jnp.exp2(s)
            l = jnp.sum(p, axis=1, keepdims=True)
            v = _unpack(v_v[2 * j + e, 0:(i + 1) * hb, :])
            o = jnp.dot(p.astype(BF16), v, preferred_element_type=F32)
            ctx_v[2 * j + e, i * hb:(i + 1) * hb, :] = _pack(o * (1.0 / l))
            mag = _tiles(jnp.maximum(jnp.abs(o), l * _TINY))
            v_new = _tiles(jnp.abs(v[i * _BQ:, :].astype(F32)))
            return (jnp.minimum(seen[0], jnp.min(mag, axis=0)),
                    jnp.maximum(seen[1], jnp.max(mag, axis=0)),
                    jnp.minimum(seen[2], jnp.min(_tiles(jnp.broadcast_to(l, o.shape)), axis=0)),
                    jnp.maximum(seen[3], jnp.max(v_new, axis=0)))

        seq = [(e, i) for t in range(nb // 2) for e in range(2) for i in (t, nb - 1 - t)]
        projected, pending = [], None
        for t, (e, i) in enumerate(seq):
            for _, soon in seq[t:t + 3]:
                if soon * _BQ // _QC not in projected:
                    projected.append(soon * _BQ // _QC)
                    q_project(projected[-1])
            s = scores(e, i)
            if pending is not None:
                seen = context(*pending, seen)
            pending = (e, i, s)
        return context(*pending, seen)

    ones = jnp.ones((8, D), F32)
    mag_lo, mag_hi, l_lo, v_hi = lax.fori_loop(0, H // 2, attention, (ones,) * 4)
    safe = ((mag_hi <= 1.0 / _TINY) & (l_lo >= _TINY) & (mag_lo >= _TINY)
            & (v_hi <= _V_MAX))

    @pl.when(jnp.max(jnp.where(safe, 0.0, 1.0)) > 0.0)
    def _true_max_attention():
        def body(t, carry):
            j, b = t // (S // _FQ), t % (S // _FQ)
            rows = pl.ds(pl.multiple_of(b * (_FQ // 2), _FQ // 2), _FQ // 2)
            q = jnp.dot(_unpack(h_v[rows, :]), _unpack(wq2_v[j]),
                        preferred_element_type=F32) * qscale
            causal = (lax.broadcasted_iota(I32, (_FQ, S), 1)
                      <= lax.broadcasted_iota(I32, (_FQ, S), 0) + b * _FQ)
            for e in range(2):
                s = lax.dot_general(q[:, e * D:(e + 1) * D].astype(BF16),
                                    _unpack(k_v[2 * j + e]), _NT, preferred_element_type=F32)
                s = jnp.where(causal, s, neg)
                p = jnp.exp2(s - jnp.max(s, axis=1, keepdims=True))
                p = p * (1.0 / jnp.sum(p, axis=1, keepdims=True))
                ctx_v[2 * j + e, rows, :] = _pack(jnp.dot(
                    p.astype(BF16), _unpack(v_v[2 * j + e]), preferred_element_type=F32))
            return carry

        lax.fori_loop(0, (H // 2) * (S // _FQ), body, 0)

    wait(tail_weights)
    wr = wr_v[...].astype(F32).reshape(1, M)
    lane = lax.broadcasted_iota(I32, (8, 128), 1)
    tiles = [jnp.zeros((8, 128), F32) for _ in range(S // 1024)]

    def second_adaln(a, att, anchor):
        att = pltpu.bitcast(_after(pltpu.bitcast(att, U32), anchor), F32)
        x1 = _rnd(x_rows(a, anchor) + _rnd(mod_v[2:3, :] * _rnd(att)))
        h2 = _adaln(x1, mod_v[3:4, :], mod_v[4:5, :])
        x1_v[a:a + _LNR, :] = x1
        h2_v[a:a + _LNR, :] = h2
        out_v[a:a + _LNR, :] = (x1 + _rnd(mod_v[5:6, :] * (h2 + h2 * 0.0))).astype(BF16)
        r = jnp.sum(h2 * wr, axis=1, keepdims=True)
        for u in range(0, _LNR, 8):
            t, ln = divmod((a + u) // 8, 128)
            tiles[t] = jnp.where(lane == ln, r[u:u + 8, :], tiles[t])

    def untranspose(src, which, f0, m0, anchor):
        n = min(128, F - f0)
        w = _unpack(_after(pltpu.bitcast(src[f0:f0 + n, m0:m0 + 128], U32), anchor))
        wgu_v[which, m0 // 2:(m0 + 128) // 2, f0:f0 + n] = _pack(w.T)

    spare = [functools.partial(untranspose, src, which, f0, m0)
             for which, src in enumerate((wg_v, wu_v))
             for f0 in range(0, F, 128) for m0 in range(0, M, 128)]
    out_copies = [
        pltpu.make_async_copy(out_v.at[pl.ds(a, n), :], out_hbm.at[pl.ds(a, n), :], out_sems.at[i])
        for i, (a, n) in enumerate(_spans(_OUT_ROWS))]
    for r0, n in _spans(_PROJ_ROWS):
        ctx = {h0: _unpack(jnp.concatenate([ctx_v[h, r0 // 2:(r0 + n) // 2, :]
                                            for h in range(h0, h0 + _OH)], axis=1))
               for h0 in range(0, H, _OH)}
        parts = []
        for c0 in range(0, M, 128):
            acc = None
            for h0 in range(0, H, _OH):
                part = jnp.dot(ctx[h0], wo_v[h0 * D:(h0 + _OH) * D, c0:c0 + 128],
                               preferred_element_type=F32)
                acc = part if acc is None else acc + part
                odd = h0 // _OH % 2
                queue = spare if spare and (odd or not jobs) else jobs
                if queue:
                    queue.pop(0)(part[0:8, :])
            parts.append(acc)
        assert not jobs
        if r0 == _OUT_ROWS[0]:
            out_copies[0].start()
        att = jnp.concatenate(parts, axis=1)
        jobs = [functools.partial(second_adaln, r0 + t, att[t:t + _LNR, :])
                for t in range(0, n, _LNR)]
    assert not spare
    for job in jobs:
        job(att[0:8, 0:128])
    out_copies[1].start()

    r = _rnd(jnp.concatenate(tiles, axis=0))
    sub = lax.broadcasted_iota(I32, r.shape, 0)
    tok = (sub // 8) * 1024 + lax.broadcasted_iota(I32, r.shape, 1) * 8 + sub % 8
    bits = pltpu.bitcast(jnp.where(r == 0.0, 0.0, r), I32) >> 16
    order = jnp.where(bits < 0, -(bits & 0x7FFF), bits) + 0x8000
    order = jnp.where(r != r, 0, order)
    key = pltpu.bitcast((order * S + (S - 1 - tok)) + 0x20000000, F32)
    idx = []
    for _ in range(_TOPC):
        top = jnp.max(jnp.max(key, axis=0, keepdims=True), axis=1, keepdims=True)
        idx.append((S - 1) - (pltpu.bitcast(top, I32)[0, 0] & (S - 1)))
        key = jnp.where(key == top, 0.0, key)

    hs = jnp.concatenate([h2_v[pl.ds(i, 1), :] for i in idx], axis=0)
    xs = jnp.concatenate([x1_v[pl.ds(i, 1), :] for i in idx], axis=0)
    hs16 = jnp.concatenate([hs, hs], axis=0).astype(BF16)
    g = _rnd(jnp.dot(hs16, _unpack(wgu_v[0]), preferred_element_type=F32))
    u = _rnd(jnp.dot(hs16, _unpack(wgu_v[1]), preferred_element_type=F32))
    act = (_rnd(g * _sigmoid(g)) * u).astype(BF16)
    y = _rnd(jnp.dot(act, wd_v[...], preferred_element_type=F32))[0:_TOPC, :]
    rs = _rnd(jnp.sum(hs * wr, axis=1, keepdims=True))
    y = _rnd(y * _sigmoid(rs))
    new = xs + _rnd(mod_v[5:6, :] * _rnd(hs + _rnd(hs * 0.0 + y)))

    wait(out_copies)
    sub16 = lax.broadcasted_iota(I32, (16, M), 0)
    groups = [pl.ds(pl.multiple_of((i // 16) * 16, 16), 16) for i in idx]
    for n, i in enumerate(idx):
        old = out_v[groups[n], :].astype(F32)
        out_v[groups[n], :] = jnp.where(sub16 == i % 16, new[n:n + 1, :], old).astype(BF16)
    fixes = []
    for n, i in enumerate(idx):
        first = True
        for prev in idx[:n]:
            first = (prev // 16 != i // 16) & first
        fixes.append((first, pltpu.make_async_copy(
            out_v.at[groups[n], :], out_hbm.at[groups[n], :], fix_sems.at[n])))
    for first, cp in fixes:
        pl.when(first)(cp.start)
    for first, cp in fixes:
        pl.when(first)(cp.wait)


@jax.jit
def pallas_adaLN_cond__compressed_kv_cla__moe_arch_mod__prompt_kernel(
    A_x: jax.Array,
    A_c_kv: jax.Array,
    A_w_q: jax.Array,
    A_w_uk: jax.Array,
    A_w_uv: jax.Array,
    A_w_o: jax.Array,
    B_x: jax.Array,
    B_w_r: jax.Array,
    B_w_gate: jax.Array,
    B_w_up: jax.Array,
    B_w_down: jax.Array,
    c: jax.Array,
    w_mod: jax.Array,
):
    del B_x
    B, S, M = A_x.shape
    Dc = A_c_kv.shape[2]
    _, H, D = A_w_q.shape
    F = B_w_down.shape[0]
    assert B == 1 and A_c_kv.shape[1] == S
    assert S == sum(_CKV_ROWS) == sum(_PROJ_ROWS) == sum(_OUT_ROWS)

    args = (
        A_x.reshape(S, M), A_c_kv.reshape(S, Dc), A_w_q, A_w_uk, A_w_uv,
        A_w_o.reshape(H * D, M), w_mod, B_w_gate.T, B_w_up.T, B_w_down, B_w_r, c,
    )
    ng = H // _HG
    scratch = [
        pltpu.VMEM((H, S // 2, D), U32),
        pltpu.VMEM((H, S // 2, D), U32),
        pltpu.VMEM((H, S // 2, D), U32),
        pltpu.VMEM((S // 2, M), U32),
        pltpu.VMEM((H // 2, M // 2, 2 * D), U32),
        pltpu.VMEM((_HG, Dc // 2, 2 * D), U32),
        pltpu.VMEM((S, M), F32),
        pltpu.VMEM((S, M), F32),
        pltpu.VMEM((S, M), BF16),
        pltpu.VMEM((_RGR * _HG // 2, D), U32),
        pltpu.VMEM((M, 128), F32),
        pltpu.VMEM((2, M // 2, F), U32),
    ] + [
        pltpu.VMEM((ng, a.shape[0], _HG, D) if a.ndim == 3 else a.shape, a.dtype)
        for a in args
    ] + [
        pltpu.VMEM((8, M), F32),
        pltpu.SemaphoreType.DMA((3 * ng + len(_CKV_ROWS) + 8,)),
        pltpu.SemaphoreType.DMA((len(_OUT_ROWS),)),
        pltpu.SemaphoreType.DMA((_TOPC,)),
    ]

    out = pl.pallas_call(
        _kernel,
        in_specs=[pl.BlockSpec(memory_space=pltpu.HBM)] * len(args),
        out_specs=pl.BlockSpec(memory_space=pltpu.HBM),
        out_shape=jax.ShapeDtypeStruct((S, M), A_x.dtype),
        scratch_shapes=scratch,
        compiler_params=pltpu.CompilerParams(vmem_limit_bytes=120 * 1024 * 1024),
        name="adaln_cla_mod",
    )(*args)
    return out.reshape(B, S, M)
```

```python
import functools
import math

import jax
import jax.numpy as jnp
from jax import lax
import jax.experimental.pallas as pl
import jax.experimental.pallas.tpu as pltpu

F32 = jnp.float32
BF16 = jnp.bfloat16
U32 = jnp.uint32
I32 = jnp.int32

_EPS = 1e-5
_TOPC = 8
_HG = 8
_KVR = 256
_LNR = 16
_RGR = 64
_MDR = 320
_QG = 32
_FQ = 256
_OH = 8
_TINY = 2.0 ** -60
_V_MAX = 2.0 ** 30
_CKV_ROWS = (256, 768, 1024)
_PROJ_ROWS = (128,) * 15 + (96, 32)
_OUT_ROWS = (1536, 512)


def _rnd(v):
    return v.astype(BF16).astype(F32)


def _adaln(x, shift, scale):
    mean = jnp.mean(x, axis=1, keepdims=True)
    d = x - mean
    var = _rnd(jnp.mean(d * d, axis=1, keepdims=True))
    den = _rnd(jnp.sqrt(_rnd(var + _rnd(jnp.full((1, 1), _EPS, F32)))))
    n = _rnd(_rnd(x - _rnd(mean)) / den)
    return _rnd(_rnd(n * _rnd(1.0 + scale)) + shift)


def _sigmoid(x):
    return _rnd(1.0 / _rnd(1.0 + _rnd(jnp.exp(-x))))


def _pack(v):
    return pltpu.bitcast(v.astype(BF16), U32)


def _unpack(v):
    return pltpu.bitcast(v, BF16)


def _after(words, anchor):
    zero = jnp.where(anchor * anchor < 0.0, jnp.uint32(1), jnp.uint32(0))
    return words | jnp.tile(zero, (words.shape[0] // 8, words.shape[1] // 128))


def _nn(a, b):
    return jnp.dot(a, b, preferred_element_type=F32)


def _nt(a, b):
    return lax.dot_general(a, b, (((1,), (1,)), ((), ())), preferred_element_type=F32)


def _tiles(v):
    return v.reshape(v.shape[0] // 8, 8, v.shape[1])


def _spans(sizes):
    out, start = [], 0
    for n in sizes:
        out.append((start, n))
        start += n
    return out


def _kernel(x_hbm, ckv_hbm, wq_hbm, wuk_hbm, wuv_hbm, wo_hbm, wmod_hbm, wg_hbm,
            wu_hbm, wd_hbm, wr_hbm, c_hbm, out_hbm,
            k_v, v_v, ctx_v, h_v, wq2_v, wkv_v, x1_v, h2_v, out_v, tmp_v, col_v, wgu_v,
            x_v, ckv_v, wq_v, wuk_v, wuv_v, wo_v, wmod_v, wg_v, wu_v, wd_v, wr_v, c_v,
            mod_v, in_sems, out_sems, fix_sems):
    (S, M), Dc, (H, _, D), F = x_v.shape, ckv_v.shape[1], k_v.shape, wd_v.shape[0]
    ng = H // _HG

    started = []

    def fetch(src, dst):
        started.append(pltpu.make_async_copy(src, dst, in_sems.at[len(started)]))
        started[-1].start()
        return started[-1]

    def fetch_group(src, dst, g):
        return fetch(src.at[:, pl.ds(g * _HG, _HG), :], dst.at[g])

    def wait(copies):
        for cp in copies:
            cp.wait()

    first_weights = fetch_group(wuk_hbm, wuk_v, 0)
    ckv_copies = {a: fetch(ckv_hbm.at[pl.ds(a, n), :], ckv_v.at[pl.ds(a, n), :])
                  for a, n in _spans(_CKV_ROWS)}
    arrivals = {
        0: [fetch_group(wuv_hbm, wuv_v, 0)],
        1: [fetch_group(wuk_hbm, wuk_v, 1), fetch_group(wuv_hbm, wuv_v, 1),
            fetch(c_hbm, c_v), fetch(wmod_hbm, wmod_v)],
        3: [fetch(x_hbm, x_v)]
           + [fetch_group(src, dst, g) for g in range(2, ng)
              for src, dst in ((wuk_hbm, wuk_v), (wuv_hbm, wuv_v))]
           + [fetch_group(wq_hbm, wq_v, g) for g in range(ng)],
    }
    tail_weights = [fetch(wo_hbm, wo_v), fetch(wr_hbm, wr_v), fetch(wg_hbm, wg_v),
                    fetch(wu_hbm, wu_v), fetch(wd_hbm, wd_v)]

    def regroup(src, g, dst, pair0, a, anchor):
        n = _RGR
        tmp_v[...] = _after(pltpu.bitcast(src[g, a:a + n].reshape(n * _HG, D), U32), anchor)
        for e in range(_HG // 2):
            w = tmp_v[pl.ds(e, n, stride=_HG // 2), :]
            dst[pair0 + e, a // 2:(a + n) // 2, 0:D] = _pack(pltpu.bitcast(w << 16, F32))
            dst[pair0 + e, a // 2:(a + n) // 2, D:2 * D] = _pack(
                pltpu.bitcast(w & jnp.uint32(0xFFFF0000), F32))

    def silu_column(anchor):
        del anchor
        cf = c_v[...].astype(F32)
        col_v[...] = jnp.broadcast_to(_rnd(cf * _sigmoid(cf)), (128, M)).T

    partial_mod = {}

    def modulation(t, a, anchor):
        w = pltpu.bitcast(wmod_v[a:a + _MDR, t:t + 128], U32)
        prod = _unpack(_after(w, anchor)).astype(F32) * col_v[a:a + _MDR, :]
        partial_mod[t] = partial_mod.get(t, 0.0) + jnp.sum(_tiles(prod), axis=0)
        if a + _MDR == M:
            mod_v[t // M:t // M + 1, t % M:t % M + 128] = _rnd(
                jnp.sum(partial_mod.pop(t), axis=0, keepdims=True))

    def x_rows(a, anchor):
        return _unpack(_after(pltpu.bitcast(x_v[a:a + _LNR, :], U32), anchor)).astype(F32)

    def first_adaln(a, anchor):
        h = _adaln(x_rows(a, anchor), mod_v[0:1, :], mod_v[1:2, :])
        h_v[a // 2:(a + _LNR) // 2, :] = _pack(h)

    released = {
        1: [silu_column] + [functools.partial(modulation, t, a)
                            for t in range(0, 6 * M, 128) for a in range(0, M, _MDR)],
        3: [functools.partial(first_adaln, a) for a in range(0, S, _LNR)]
           + [functools.partial(regroup, wq_v, g, wq2_v, g * (_HG // 2), a)
              for g in range(ng) for a in range(0, M, _RGR)],
    }
    stages = [(src, g, o_v) for g in range(ng) for src, o_v in ((wuk_v, k_v), (wuv_v, v_v))]
    jobs = []
    first_weights.wait()
    for t, (src, g, o_v) in enumerate(stages):
        for r0 in range(0, S, _KVR):
            if t == 0 and r0 in ckv_copies:
                ckv_copies[r0].wait()
                if r0 == 0:
                    w0 = src[g].reshape(Dc, _HG * D)
            if r0 == S // 2 and t + 1 < len(stages):
                wait(arrivals.get(t, []))
                jobs = [functools.partial(regroup, *stages[t + 1][:2], wkv_v,
                                          (t + 1) % 2 * (_HG // 2), a)
                        for a in range(0, Dc, _RGR)] + jobs + released.get(t, [])
            for e0 in range(0, _HG, 4):
                if t == 0:
                    w = w0[:, e0 * D:(e0 + 4) * D]
                else:
                    w = jnp.concatenate([_unpack(wkv_v[t % 2 * (_HG // 2) + e0 // 2 + e])
                                         for e in range(2)], axis=1)
                r = _nn(ckv_v[r0:r0 + _KVR, :], w)
                for e in range(4):
                    head = r[:, e * D:(e + 1) * D]
                    o_v[g * _HG + e0 + e, r0 // 2:(r0 + _KVR) // 2, :] = _pack(head)
                    if jobs:
                        jobs.pop(0)(head[0:8, :])
    assert not jobs

    qscale = float(D ** -0.5 * math.log2(math.e))
    neg = float(-1e9 * math.log2(math.e))
    nu = 128 // _QG
    panel = 128 * nu

    def attention(j, seen):
        tri = (lax.broadcasted_iota(I32, (_QG, 128), 1)
               <= lax.broadcasted_iota(I32, (_QG, 128), 0) + (128 - _QG))
        zero = (j >> 16).astype(U32)
        qs, finished = {}, []

        def keys(ref, e, a, b):
            return _unpack(ref[2 * j + e, a // 2:b // 2, :])

        def on_diagonal(s):
            top = jnp.where(tri, s[:_QG], neg)
            return jnp.concatenate([top, s[_QG:]], 0) if s.shape[0] > _QG else top

        def q_project(c):
            hc = _unpack(h_v[c * panel // 2:(c + 1) * panel // 2, :])
            q = _nn(hc, _unpack(wq2_v[j])) * qscale
            for e in range(2):
                for u in range(nu):
                    qs[e, c, u] = _pack(jnp.concatenate(
                        [q[t:t + _QG, e * D:(e + 1) * D] for t in range(u * _QG, panel, 128)], 0))

        def scores(e, c, u):
            q = qs.pop((e, c, u))
            if len(finished) >= 3:
                q = q | (finished.pop(0) & zero)
            q = _unpack(q)
            lead, end = (u + 1) * _QG % 128, c * panel + (u + 1) * _QG
            head = body = None
            if lead:
                head = _nt(keys(k_v, e, 0, lead), q)
                if c == 0:
                    head = jnp.where(lax.broadcasted_iota(I32, head.shape, 0) - u * _QG
                                     <= lax.broadcasted_iota(I32, head.shape, 1), head, neg)
            if end > lead:
                body = _nt(q, keys(k_v, e, lead, end))
                last = on_diagonal(body[:, -128:])
                body = jnp.concatenate([body[:, :-128], last], 1) if end - lead > 128 else last
            steps = [on_diagonal(_nt(q[t * _QG:], keys(k_v, e, end + 128 * (t - 1), end + 128 * t)))
                     for t in range(1, nu)]
            return head, body, steps

        def context(e, c, u, head, body, steps, seen):
            lead, end = (u + 1) * _QG % 128, c * panel + (u + 1) * _QG
            ls, accs = [], []
            if body is not None:
                p = jnp.exp2(body)
                ls += [p[:, t:t + 128] for t in range(0, end - lead, 128)]
                accs.append(_nn(p.astype(BF16), keys(v_v, e, lead, end)))
            if head is not None:
                p = jnp.concatenate([jnp.exp2(head), jnp.zeros((128 - lead, 128), F32)], 0).T
                ls.append(p)
                accs.append(_nn(p.astype(BF16), keys(v_v, e, 0, 128)))
            l, o = functools.reduce(jnp.add, ls), functools.reduce(jnp.add, accs)
            for t, s in enumerate(steps, 1):
                p = jnp.exp2(s)
                pv = _nn(p.astype(BF16), keys(v_v, e, end + 128 * (t - 1), end + 128 * t))
                l = jnp.concatenate([l[:t * _QG], l[t * _QG:] + p], 0)
                o = jnp.concatenate([o[:t * _QG], o[t * _QG:] + pv], 0)
            l = jnp.sum(l, axis=1, keepdims=True)
            ctx = _pack(o * (1.0 / l))
            for t in range(nu):
                a = c * panel + 128 * t + u * _QG
                ctx_v[2 * j + e, a // 2:(a + _QG) // 2, :] = ctx[t * _QG // 2:(t + 1) * _QG // 2]
            mag = _tiles(jnp.maximum(jnp.abs(o), l * _TINY))
            a = c * panel + 128 * u
            v = _unpack(v_v[2 * j + e, a // 2:(a + 128) // 2, :] | (ctx & zero))
            seen = (jnp.minimum(seen[0], jnp.min(mag, axis=0)),
                    jnp.maximum(seen[1], jnp.max(mag, axis=0)),
                    jnp.minimum(seen[2], jnp.min(_tiles(jnp.broadcast_to(l, o.shape)), axis=0)),
                    jnp.maximum(seen[3], jnp.max(_tiles(jnp.abs(v.astype(F32))), axis=0)))
            finished.append(
                ctx | jnp.tile(pltpu.bitcast(functools.reduce(jnp.add, seen), U32), (8, 1)))
            return seen

        seq = [(e, c, u) for t in range(S // panel // 2) for e in range(2) for u in range(nu)
               for c in (t, S // panel - 1 - t)]
        projected, pending = [], []
        for t, block in enumerate(seq):
            for _, c, _ in seq[t:t + 3]:
                if c not in projected:
                    projected.append(c)
                    q_project(c)
            pending.append(block + scores(*block))
            if len(pending) > 2:
                seen = context(*pending.pop(0), seen)
        for block in pending:
            seen = context(*block, seen)
        return seen

    ones = jnp.ones((8, D), F32)
    mag_lo, mag_hi, l_lo, v_hi = lax.fori_loop(0, H // 2, attention, (ones,) * 4)
    safe = ((mag_hi <= 1.0 / _TINY) & (l_lo >= _TINY) & (mag_lo >= _TINY)
            & (v_hi <= _V_MAX))

    @pl.when(jnp.max(jnp.where(safe, 0.0, 1.0)) > 0.0)
    def _true_max_attention():
        def body(t, carry):
            j, b = t // (S // _FQ), t % (S // _FQ)
            rows = pl.ds(pl.multiple_of(b * (_FQ // 2), _FQ // 2), _FQ // 2)
            q = _nn(_unpack(h_v[rows, :]), _unpack(wq2_v[j])) * qscale
            causal = (lax.broadcasted_iota(I32, (_FQ, S), 1)
                      <= lax.broadcasted_iota(I32, (_FQ, S), 0) + b * _FQ)
            for e in range(2):
                s = _nt(q[:, e * D:(e + 1) * D].astype(BF16), _unpack(k_v[2 * j + e]))
                s = jnp.where(causal, s, neg)
                p = jnp.exp2(s - jnp.max(s, axis=1, keepdims=True))
                p = p * (1.0 / jnp.sum(p, axis=1, keepdims=True))
                ctx_v[2 * j + e, rows, :] = _pack(_nn(p.astype(BF16), _unpack(v_v[2 * j + e])))
            return carry

        lax.fori_loop(0, (H // 2) * (S // _FQ), body, 0)

    wait(tail_weights)
    wr = wr_v[...].astype(F32).reshape(1, M)
    lane = lax.broadcasted_iota(I32, (8, 128), 1)
    tiles = [jnp.zeros((8, 128), F32) for _ in range(S // 1024)]

    def second_adaln(a, att, anchor):
        att = pltpu.bitcast(_after(pltpu.bitcast(att, U32), anchor), F32)
        x1 = _rnd(x_rows(a, anchor) + _rnd(mod_v[2:3, :] * _rnd(att)))
        h2 = _adaln(x1, mod_v[3:4, :], mod_v[4:5, :])
        x1_v[a:a + _LNR, :] = x1
        h2_v[a:a + _LNR, :] = h2
        out_v[a:a + _LNR, :] = (x1 + _rnd(mod_v[5:6, :] * (h2 + h2 * 0.0))).astype(BF16)
        r = jnp.sum(h2 * wr, axis=1, keepdims=True)
        for u in range(0, _LNR, 8):
            t, ln = divmod((a + u) // 8, 128)
            tiles[t] = jnp.where(lane == ln, r[u:u + 8, :], tiles[t])

    def untranspose(src, which, f0, m0, anchor):
        n = min(128, F - f0)
        w = _unpack(_after(pltpu.bitcast(src[f0:f0 + n, m0:m0 + 128], U32), anchor))
        wgu_v[which, m0 // 2:(m0 + 128) // 2, f0:f0 + n] = _pack(w.T)

    spare = [functools.partial(untranspose, src, which, f0, m0)
             for which, src in enumerate((wg_v, wu_v))
             for f0 in range(0, F, 128) for m0 in range(0, M, 128)]
    out_copies = [
        pltpu.make_async_copy(out_v.at[pl.ds(a, n), :], out_hbm.at[pl.ds(a, n), :], out_sems.at[i])
        for i, (a, n) in enumerate(_spans(_OUT_ROWS))]
    for r0, n in _spans(_PROJ_ROWS):
        ctx = {h0: _unpack(jnp.concatenate([ctx_v[h, r0 // 2:(r0 + n) // 2, :]
                                            for h in range(h0, h0 + _OH)], axis=1))
               for h0 in range(0, H, _OH)}
        parts = []
        for c0 in range(0, M, 128):
            acc = None
            for h0 in range(0, H, _OH):
                part = _nn(ctx[h0], wo_v[h0 * D:(h0 + _OH) * D, c0:c0 + 128])
                acc = part if acc is None else acc + part
                odd = h0 // _OH % 2
                queue = spare if spare and (odd or not jobs) else jobs
                if queue:
                    queue.pop(0)(part[0:8, :])
            parts.append(acc)
        assert not jobs
        if r0 == _OUT_ROWS[0]:
            out_copies[0].start()
        att = jnp.concatenate(parts, axis=1)
        jobs = [functools.partial(second_adaln, r0 + t, att[t:t + _LNR, :])
                for t in range(0, n, _LNR)]
    assert not spare
    for job in jobs:
        job(att[0:8, 0:128])
    out_copies[1].start()

    r = _rnd(jnp.concatenate(tiles, axis=0))
    sub = lax.broadcasted_iota(I32, r.shape, 0)
    tok = (sub // 8) * 1024 + lax.broadcasted_iota(I32, r.shape, 1) * 8 + sub % 8
    bits = pltpu.bitcast(jnp.where(r == 0.0, 0.0, r), I32) >> 16
    order = jnp.where(bits < 0, -(bits & 0x7FFF), bits) + 0x8000
    order = jnp.where(r != r, 0, order)
    key = pltpu.bitcast((order * S + (S - 1 - tok)) + 0x20000000, F32)
    idx = []
    for _ in range(_TOPC):
        top = jnp.max(jnp.max(key, axis=0, keepdims=True), axis=1, keepdims=True)
        idx.append((S - 1) - (pltpu.bitcast(top, I32)[0, 0] & (S - 1)))
        key = jnp.where(key == top, 0.0, key)

    hs = jnp.concatenate([h2_v[pl.ds(i, 1), :] for i in idx], axis=0)
    xs = jnp.concatenate([x1_v[pl.ds(i, 1), :] for i in idx], axis=0)
    hs16 = jnp.concatenate([hs, hs], axis=0).astype(BF16)
    g = _rnd(_nn(hs16, _unpack(wgu_v[0])))
    u = _rnd(_nn(hs16, _unpack(wgu_v[1])))
    act = (_rnd(g * _sigmoid(g)) * u).astype(BF16)
    y = _rnd(_nn(act, wd_v[...]))[0:_TOPC, :]
    rs = _rnd(jnp.sum(hs * wr, axis=1, keepdims=True))
    y = _rnd(y * _sigmoid(rs))
    new = xs + _rnd(mod_v[5:6, :] * _rnd(hs + _rnd(hs * 0.0 + y)))

    wait(out_copies)
    sub16 = lax.broadcasted_iota(I32, (16, M), 0)
    groups = [pl.ds(pl.multiple_of((i // 16) * 16, 16), 16) for i in idx]
    for n, i in enumerate(idx):
        old = out_v[groups[n], :].astype(F32)
        out_v[groups[n], :] = jnp.where(sub16 == i % 16, new[n:n + 1, :], old).astype(BF16)
    fixes = []
    for n, i in enumerate(idx):
        first = True
        for prev in idx[:n]:
            first = (prev // 16 != i // 16) & first
        fixes.append((first, pltpu.make_async_copy(
            out_v.at[groups[n], :], out_hbm.at[groups[n], :], fix_sems.at[n])))
    for first, cp in fixes:
        pl.when(first)(cp.start)
    for first, cp in fixes:
        pl.when(first)(cp.wait)


@jax.jit
def pallas_adaLN_cond__compressed_kv_cla__moe_arch_mod__prompt_kernel(
    A_x: jax.Array,
    A_c_kv: jax.Array,
    A_w_q: jax.Array,
    A_w_uk: jax.Array,
    A_w_uv: jax.Array,
    A_w_o: jax.Array,
    B_x: jax.Array,
    B_w_r: jax.Array,
    B_w_gate: jax.Array,
    B_w_up: jax.Array,
    B_w_down: jax.Array,
    c: jax.Array,
    w_mod: jax.Array,
):
    del B_x
    B, S, M = A_x.shape
    Dc = A_c_kv.shape[2]
    _, H, D = A_w_q.shape
    F = B_w_down.shape[0]
    assert B == 1 and A_c_kv.shape[1] == S
    assert S == sum(_CKV_ROWS) == sum(_PROJ_ROWS) == sum(_OUT_ROWS)

    args = (
        A_x.reshape(S, M), A_c_kv.reshape(S, Dc), A_w_q, A_w_uk, A_w_uv,
        A_w_o.reshape(H * D, M), w_mod, B_w_gate.T, B_w_up.T, B_w_down, B_w_r, c,
    )
    ng = H // _HG
    scratch = [
        pltpu.VMEM((H, S // 2, D), U32),
        pltpu.VMEM((H, S // 2, D), U32),
        pltpu.VMEM((H, S // 2, D), U32),
        pltpu.VMEM((S // 2, M), U32),
        pltpu.VMEM((H // 2, M // 2, 2 * D), U32),
        pltpu.VMEM((_HG, Dc // 2, 2 * D), U32),
        pltpu.VMEM((S, M), F32),
        pltpu.VMEM((S, M), F32),
        pltpu.VMEM((S, M), BF16),
        pltpu.VMEM((_RGR * _HG // 2, D), U32),
        pltpu.VMEM((M, 128), F32),
        pltpu.VMEM((2, M // 2, F), U32),
    ] + [
        pltpu.VMEM((ng, a.shape[0], _HG, D) if a.ndim == 3 else a.shape, a.dtype)
        for a in args
    ] + [
        pltpu.VMEM((8, M), F32),
        pltpu.SemaphoreType.DMA((3 * ng + len(_CKV_ROWS) + 8,)),
        pltpu.SemaphoreType.DMA((len(_OUT_ROWS),)),
        pltpu.SemaphoreType.DMA((_TOPC,)),
    ]

    out = pl.pallas_call(
        _kernel,
        in_specs=[pl.BlockSpec(memory_space=pltpu.HBM)] * len(args),
        out_specs=pl.BlockSpec(memory_space=pltpu.HBM),
        out_shape=jax.ShapeDtypeStruct((S, M), A_x.dtype),
        scratch_shapes=scratch,
        compiler_params=pltpu.CompilerParams(vmem_limit_bytes=120 * 1024 * 1024),
        name="adaln_cla_mod",
    )(*args)
    return out.reshape(B, S, M)
```

```python
import functools
import math

import jax
import jax.numpy as jnp
from jax import lax
import jax.experimental.pallas as pl
import jax.experimental.pallas.tpu as pltpu

F32 = jnp.float32
BF16 = jnp.bfloat16
U32 = jnp.uint32
I32 = jnp.int32

_EPS = 1e-5
_TOPC = 8
_HG = 8
_KVR = 256
_LNR = 16
_RGR = 64
_MDR = 320
_QG = 32
_FQ = 256
_OH = 8
_TINY = 2.0 ** -60
_V_MAX = 2.0 ** 30
_CKV_ROWS = (256, 512, 1280)
_PROJ_ROWS = (128,) * 15 + (96, 32)
_OUT_ROWS = (1536, 512)


def _rnd(v):
    return v.astype(BF16).astype(F32)


def _adaln(x, shift, scale):
    mean = jnp.mean(x, axis=1, keepdims=True)
    d = x - mean
    var = _rnd(jnp.mean(d * d, axis=1, keepdims=True))
    den = _rnd(jnp.sqrt(_rnd(var + _rnd(jnp.full((1, 1), _EPS, F32)))))
    n = _rnd(_rnd(x - _rnd(mean)) / den)
    return _rnd(_rnd(n * _rnd(1.0 + scale)) + shift)


def _sigmoid(x):
    return _rnd(1.0 / _rnd(1.0 + _rnd(jnp.exp(-x))))


def _pack(v):
    return pltpu.bitcast(v.astype(BF16), U32)


def _unpack(v):
    return pltpu.bitcast(v, BF16)


def _after(words, anchor):
    zero = jnp.where(anchor * anchor < 0.0, jnp.uint32(1), jnp.uint32(0))
    return words | jnp.tile(zero, (words.shape[0] // 8, words.shape[1] // 128))


def _nn(a, b):
    return jnp.dot(a, b, preferred_element_type=F32)


def _nt(a, b):
    return lax.dot_general(a, b, (((1,), (1,)), ((), ())), preferred_element_type=F32)


def _tiles(v):
    return v.reshape(v.shape[0] // 8, 8, v.shape[1])


def _spans(sizes):
    out, start = [], 0
    for n in sizes:
        out.append((start, n))
        start += n
    return out


def _kernel(x_hbm, ckv_hbm, wq_hbm, wuk_hbm, wuv_hbm, wo_hbm, wmod_hbm, wg_hbm,
            wu_hbm, wd_hbm, wr_hbm, c_hbm, out_hbm,
            k_v, v_v, ctx_v, h_v, wq2_v, wkv_v, x1_v, h2_v, out_v, tmp_v, col_v, wgu_v,
            x_v, ckv_v, wq_v, wuk_v, wuv_v, wo_v, wmod_v, wg_v, wu_v, wd_v, wr_v, c_v,
            mod_v, in_sems, out_sems, fix_sems):
    (S, M), Dc, (H, _, D), F = x_v.shape, ckv_v.shape[1], k_v.shape, wd_v.shape[0]
    ng = H // _HG

    started = []

    def fetch(src, dst):
        started.append(pltpu.make_async_copy(src, dst, in_sems.at[len(started)]))
        started[-1].start()
        return started[-1]

    def fetch_group(src, dst, g):
        return fetch(src.at[:, pl.ds(g * _HG, _HG), :], dst.at[g])

    def wait(copies):
        for cp in copies:
            cp.wait()

    def fetch_ckv(a, n):
        return fetch(ckv_hbm.at[pl.ds(a, n), :], ckv_v.at[pl.ds(a, n), :])

    def fetch_first_weights(a):
        return fetch(wuk_hbm.at[pl.ds(a, Dc // 2), pl.ds(0, _HG), :],
                     wuk_v.at[0, pl.ds(a, Dc // 2)])

    opening = [fetch_first_weights(0), fetch_ckv(0, _CKV_ROWS[0])]
    first_stage = {0: fetch_first_weights(Dc // 2)}
    first_stage.update({a: fetch_ckv(a, n) for a, n in _spans(_CKV_ROWS)[1:]})
    arrivals = {
        0: [fetch_group(wuv_hbm, wuv_v, 0)],
        1: [fetch_group(wuk_hbm, wuk_v, 1), fetch_group(wuv_hbm, wuv_v, 1),
            fetch(c_hbm, c_v), fetch(wmod_hbm, wmod_v)],
        3: [fetch(x_hbm, x_v)]
           + [fetch_group(src, dst, g) for g in range(2, ng)
              for src, dst in ((wuk_hbm, wuk_v), (wuv_hbm, wuv_v))]
           + [fetch_group(wq_hbm, wq_v, g) for g in range(ng)],
    }
    tail_weights = [fetch(wo_hbm, wo_v), fetch(wr_hbm, wr_v), fetch(wg_hbm, wg_v),
                    fetch(wu_hbm, wu_v), fetch(wd_hbm, wd_v)]

    def regroup(src, g, dst, pair0, a, anchor):
        n = _RGR
        tmp_v[...] = _after(pltpu.bitcast(src[g, a:a + n].reshape(n * _HG, D), U32), anchor)
        for e in range(_HG // 2):
            w = tmp_v[pl.ds(e, n, stride=_HG // 2), :]
            dst[pair0 + e, a // 2:(a + n) // 2, 0:D] = _pack(pltpu.bitcast(w << 16, F32))
            dst[pair0 + e, a // 2:(a + n) // 2, D:2 * D] = _pack(
                pltpu.bitcast(w & jnp.uint32(0xFFFF0000), F32))

    def silu_column(anchor):
        del anchor
        cf = c_v[...].astype(F32)
        col_v[...] = jnp.broadcast_to(_rnd(cf * _sigmoid(cf)), (128, M)).T

    partial_mod = {}

    def modulation(t, a, anchor):
        w = pltpu.bitcast(wmod_v[a:a + _MDR, t:t + 128], U32)
        prod = _unpack(_after(w, anchor)).astype(F32) * col_v[a:a + _MDR, :]
        partial_mod[t] = partial_mod.get(t, 0.0) + jnp.sum(_tiles(prod), axis=0)
        if a + _MDR == M:
            mod_v[t // M:t // M + 1, t % M:t % M + 128] = _rnd(
                jnp.sum(partial_mod.pop(t), axis=0, keepdims=True))

    def x_rows(a, anchor):
        return _unpack(_after(pltpu.bitcast(x_v[a:a + _LNR, :], U32), anchor)).astype(F32)

    def first_adaln(a, anchor):
        h = _adaln(x_rows(a, anchor), mod_v[0:1, :], mod_v[1:2, :])
        h_v[a // 2:(a + _LNR) // 2, :] = _pack(h)

    released = {
        1: [silu_column] + [functools.partial(modulation, t, a)
                            for t in range(0, 6 * M, 128) for a in range(0, M, _MDR)],
        3: [functools.partial(first_adaln, a) for a in range(0, S, _LNR)]
           + [functools.partial(regroup, wq_v, g, wq2_v, g * (_HG // 2), a)
              for g in range(ng) for a in range(0, M, _RGR)],
    }
    stages = [(src, g, o_v) for g in range(ng) for src, o_v in ((wuk_v, k_v), (wuv_v, v_v))]
    jobs = []
    wait(opening)
    w0 = wuk_v[0, 0:Dc // 2].reshape(Dc // 2, _HG * D)
    half = _nn(ckv_v[0:_KVR, 0:Dc // 2], w0)
    for t, (_, g, o_v) in enumerate(stages):
        for r0 in range(0, S, _KVR):
            if t == 0 and r0 in first_stage:
                first_stage[r0].wait()
                if r0 == 0:
                    w0 = jnp.concatenate(
                        [w0, wuk_v[0, Dc // 2:Dc].reshape(Dc // 2, _HG * D)], axis=0)
            if r0 == S // 2 and t + 1 < len(stages):
                wait(arrivals.get(t, []))
                jobs = [functools.partial(regroup, *stages[t + 1][:2], wkv_v,
                                          (t + 1) % 2 * (_HG // 2), a)
                        for a in range(0, Dc, _RGR)] + jobs + released.get(t, [])
            for e0 in range(0, _HG, 4):
                if t == 0:
                    w = w0[:, e0 * D:(e0 + 4) * D]
                else:
                    w = jnp.concatenate([_unpack(wkv_v[t % 2 * (_HG // 2) + e0 // 2 + e])
                                         for e in range(2)], axis=1)
                if t == 0 and r0 == 0:
                    r = half[:, e0 * D:(e0 + 4) * D] + _nn(ckv_v[0:_KVR, Dc // 2:Dc], w[Dc // 2:])
                else:
                    r = _nn(ckv_v[r0:r0 + _KVR, :], w)
                for e in range(4):
                    head = r[:, e * D:(e + 1) * D]
                    o_v[g * _HG + e0 + e, r0 // 2:(r0 + _KVR) // 2, :] = _pack(head)
                    if jobs:
                        jobs.pop(0)(head[0:8, :])
    assert not jobs

    qscale = float(D ** -0.5 * math.log2(math.e))
    neg = float(-1e9 * math.log2(math.e))
    nu = 128 // _QG
    panel = 128 * nu

    def attention(j, seen):
        tri = (lax.broadcasted_iota(I32, (_QG, 128), 1)
               <= lax.broadcasted_iota(I32, (_QG, 128), 0) + (128 - _QG))
        zero = (j >> 16).astype(U32)
        qs, finished = {}, []

        def keys(ref, e, a, b):
            return _unpack(ref[2 * j + e, a // 2:b // 2, :])

        def on_diagonal(s):
            top = jnp.where(tri, s[:_QG], neg)
            return jnp.concatenate([top, s[_QG:]], 0) if s.shape[0] > _QG else top

        def q_project(c):
            hc = _unpack(h_v[c * panel // 2:(c + 1) * panel // 2, :])
            q = _nn(hc, _unpack(wq2_v[j])) * qscale
            for e in range(2):
                for u in range(nu):
                    qs[e, c, u] = _pack(jnp.concatenate(
                        [q[t:t + _QG, e * D:(e + 1) * D] for t in range(u * _QG, panel, 128)], 0))

        def scores(e, c, u):
            q = qs.pop((e, c, u))
            if len(finished) >= 3:
                q = q | (finished.pop(0) & zero)
            q = _unpack(q)
            lead, end = (u + 1) * _QG % 128, c * panel + (u + 1) * _QG
            head = body = None
            if lead:
                head = _nt(keys(k_v, e, 0, lead), q)
                if c == 0:
                    head = jnp.where(lax.broadcasted_iota(I32, head.shape, 0) - u * _QG
                                     <= lax.broadcasted_iota(I32, head.shape, 1), head, neg)
            if end > lead:
                body = _nt(q, keys(k_v, e, lead, end))
                last = on_diagonal(body[:, -128:])
                body = jnp.concatenate([body[:, :-128], last], 1) if end - lead > 128 else last
            steps = [on_diagonal(_nt(q[t * _QG:], keys(k_v, e, end + 128 * (t - 1), end + 128 * t)))
                     for t in range(1, nu)]
            return head, body, steps

        def context(e, c, u, head, body, steps, seen):
            lead, end = (u + 1) * _QG % 128, c * panel + (u + 1) * _QG
            ls, accs = [], []
            if body is not None:
                p = jnp.exp2(body)
                ls += [p[:, t:t + 128] for t in range(0, end - lead, 128)]
                accs.append(_nn(p.astype(BF16), keys(v_v, e, lead, end)))
            if head is not None:
                p = jnp.concatenate([jnp.exp2(head), jnp.zeros((128 - lead, 128), F32)], 0).T
                ls.append(p)
                accs.append(_nn(p.astype(BF16), keys(v_v, e, 0, 128)))
            l, o = functools.reduce(jnp.add, ls), functools.reduce(jnp.add, accs)
            for t, s in enumerate(steps, 1):
                p = jnp.exp2(s)
                pv = _nn(p.astype(BF16), keys(v_v, e, end + 128 * (t - 1), end + 128 * t))
                l = jnp.concatenate([l[:t * _QG], l[t * _QG:] + p], 0)
                o = jnp.concatenate([o[:t * _QG], o[t * _QG:] + pv], 0)
            l = jnp.sum(l, axis=1, keepdims=True)
            ctx = _pack(o * (1.0 / l))
            for t in range(nu):
                a = c * panel + 128 * t + u * _QG
                ctx_v[2 * j + e, a // 2:(a + _QG) // 2, :] = ctx[t * _QG // 2:(t + 1) * _QG // 2]
            mag = _tiles(jnp.maximum(jnp.abs(o), l * _TINY))
            a = c * panel + 128 * u
            v = _unpack(v_v[2 * j + e, a // 2:(a + 128) // 2, :] | (ctx & zero))
            seen = (jnp.minimum(seen[0], jnp.min(mag, axis=0)),
                    jnp.maximum(seen[1], jnp.max(mag, axis=0)),
                    jnp.minimum(seen[2], jnp.min(_tiles(jnp.broadcast_to(l, o.shape)), axis=0)),
                    jnp.maximum(seen[3], jnp.max(_tiles(jnp.abs(v.astype(F32))), axis=0)))
            finished.append(
                ctx | jnp.tile(pltpu.bitcast(functools.reduce(jnp.add, seen), U32), (8, 1)))
            return seen

        seq = [(e, c, u) for t in range(S // panel // 2) for e in range(2) for u in range(nu)
               for c in (t, S // panel - 1 - t)]
        projected, pending = [], []
        for t, block in enumerate(seq):
            for _, c, _ in seq[t:t + 3]:
                if c not in projected:
                    projected.append(c)
                    q_project(c)
            pending.append(block + scores(*block))
            if len(pending) > 2:
                seen = context(*pending.pop(0), seen)
        for block in pending:
            seen = context(*block, seen)
        return seen

    ones = jnp.ones((8, D), F32)
    mag_lo, mag_hi, l_lo, v_hi = lax.fori_loop(0, H // 2, attention, (ones,) * 4)
    safe = ((mag_hi <= 1.0 / _TINY) & (l_lo >= _TINY) & (mag_lo >= _TINY)
            & (v_hi <= _V_MAX))

    @pl.when(jnp.max(jnp.where(safe, 0.0, 1.0)) > 0.0)
    def _true_max_attention():
        def body(t, carry):
            j, b = t // (S // _FQ), t % (S // _FQ)
            rows = pl.ds(pl.multiple_of(b * (_FQ // 2), _FQ // 2), _FQ // 2)
            q = _nn(_unpack(h_v[rows, :]), _unpack(wq2_v[j])) * qscale
            causal = (lax.broadcasted_iota(I32, (_FQ, S), 1)
                      <= lax.broadcasted_iota(I32, (_FQ, S), 0) + b * _FQ)
            for e in range(2):
                s = _nt(q[:, e * D:(e + 1) * D].astype(BF16), _unpack(k_v[2 * j + e]))
                s = jnp.where(causal, s, neg)
                p = jnp.exp2(s - jnp.max(s, axis=1, keepdims=True))
                p = p * (1.0 / jnp.sum(p, axis=1, keepdims=True))
                ctx_v[2 * j + e, rows, :] = _pack(_nn(p.astype(BF16), _unpack(v_v[2 * j + e])))
            return carry

        lax.fori_loop(0, (H // 2) * (S // _FQ), body, 0)

    wait(tail_weights)
    wr = wr_v[...].astype(F32).reshape(1, M)
    lane = lax.broadcasted_iota(I32, (8, 128), 1)
    tiles = [jnp.zeros((8, 128), F32) for _ in range(S // 1024)]

    def second_adaln(a, att, anchor):
        att = pltpu.bitcast(_after(pltpu.bitcast(att, U32), anchor), F32)
        x1 = _rnd(x_rows(a, anchor) + _rnd(mod_v[2:3, :] * _rnd(att)))
        h2 = _adaln(x1, mod_v[3:4, :], mod_v[4:5, :])
        x1_v[a:a + _LNR, :] = x1
        h2_v[a:a + _LNR, :] = h2
        out_v[a:a + _LNR, :] = (x1 + _rnd(mod_v[5:6, :] * (h2 + h2 * 0.0))).astype(BF16)
        r = jnp.sum(h2 * wr, axis=1, keepdims=True)
        for u in range(0, _LNR, 8):
            t, ln = divmod((a + u) // 8, 128)
            tiles[t] = jnp.where(lane == ln, r[u:u + 8, :], tiles[t])

    def untranspose(src, which, f0, m0, anchor):
        n = min(128, F - f0)
        w = _unpack(_after(pltpu.bitcast(src[f0:f0 + n, m0:m0 + 128], U32), anchor))
        wgu_v[which, m0 // 2:(m0 + 128) // 2, f0:f0 + n] = _pack(w.T)

    spare = [functools.partial(untranspose, src, which, f0, m0)
             for which, src in enumerate((wg_v, wu_v))
             for f0 in range(0, F, 128) for m0 in range(0, M, 128)]
    out_copies = [
        pltpu.make_async_copy(out_v.at[pl.ds(a, n), :], out_hbm.at[pl.ds(a, n), :], out_sems.at[i])
        for i, (a, n) in enumerate(_spans(_OUT_ROWS))]
    for r0, n in _spans(_PROJ_ROWS):
        ctx = {h0: _unpack(jnp.concatenate([ctx_v[h, r0 // 2:(r0 + n) // 2, :]
                                            for h in range(h0, h0 + _OH)], axis=1))
               for h0 in range(0, H, _OH)}
        parts = []
        for c0 in range(0, M, 128):
            acc = None
            for h0 in range(0, H, _OH):
                part = _nn(ctx[h0], wo_v[h0 * D:(h0 + _OH) * D, c0:c0 + 128])
                acc = part if acc is None else acc + part
                odd = h0 // _OH % 2
                queue = spare if spare and (odd or not jobs) else jobs
                if queue:
                    queue.pop(0)(part[0:8, :])
            parts.append(acc)
        assert not jobs
        if r0 == _OUT_ROWS[0]:
            out_copies[0].start()
        att = jnp.concatenate(parts, axis=1)
        jobs = [functools.partial(second_adaln, r0 + t, att[t:t + _LNR, :])
                for t in range(0, n, _LNR)]
    assert not spare
    for job in jobs:
        job(att[0:8, 0:128])
    out_copies[1].start()

    r = _rnd(jnp.concatenate(tiles, axis=0))
    sub = lax.broadcasted_iota(I32, r.shape, 0)
    tok = (sub // 8) * 1024 + lax.broadcasted_iota(I32, r.shape, 1) * 8 + sub % 8
    bits = pltpu.bitcast(jnp.where(r == 0.0, 0.0, r), I32) >> 16
    order = jnp.where(bits < 0, -(bits & 0x7FFF), bits) + 0x8000
    order = jnp.where(r != r, 0, order)
    key = pltpu.bitcast((order * S + (S - 1 - tok)) + 0x20000000, F32)
    idx = []
    for _ in range(_TOPC):
        top = jnp.max(jnp.max(key, axis=0, keepdims=True), axis=1, keepdims=True)
        idx.append((S - 1) - (pltpu.bitcast(top, I32)[0, 0] & (S - 1)))
        key = jnp.where(key == top, 0.0, key)

    hs = jnp.concatenate([h2_v[pl.ds(i, 1), :] for i in idx], axis=0)
    xs = jnp.concatenate([x1_v[pl.ds(i, 1), :] for i in idx], axis=0)
    hs16 = jnp.concatenate([hs, hs], axis=0).astype(BF16)
    g = _rnd(_nn(hs16, _unpack(wgu_v[0])))
    u = _rnd(_nn(hs16, _unpack(wgu_v[1])))
    act = (_rnd(g * _sigmoid(g)) * u).astype(BF16)
    y = _rnd(_nn(act, wd_v[...]))[0:_TOPC, :]
    rs = _rnd(jnp.sum(hs * wr, axis=1, keepdims=True))
    y = _rnd(y * _sigmoid(rs))
    new = xs + _rnd(mod_v[5:6, :] * _rnd(hs + _rnd(hs * 0.0 + y)))

    wait(out_copies)
    sub16 = lax.broadcasted_iota(I32, (16, M), 0)
    groups = [pl.ds(pl.multiple_of((i // 16) * 16, 16), 16) for i in idx]
    for n, i in enumerate(idx):
        old = out_v[groups[n], :].astype(F32)
        out_v[groups[n], :] = jnp.where(sub16 == i % 16, new[n:n + 1, :], old).astype(BF16)
    fixes = []
    for n, i in enumerate(idx):
        first = True
        for prev in idx[:n]:
            first = (prev // 16 != i // 16) & first
        fixes.append((first, pltpu.make_async_copy(
            out_v.at[groups[n], :], out_hbm.at[groups[n], :], fix_sems.at[n])))
    for first, cp in fixes:
        pl.when(first)(cp.start)
    for first, cp in fixes:
        pl.when(first)(cp.wait)


@jax.jit
def pallas_adaLN_cond__compressed_kv_cla__moe_arch_mod__prompt_kernel(
    A_x: jax.Array,
    A_c_kv: jax.Array,
    A_w_q: jax.Array,
    A_w_uk: jax.Array,
    A_w_uv: jax.Array,
    A_w_o: jax.Array,
    B_x: jax.Array,
    B_w_r: jax.Array,
    B_w_gate: jax.Array,
    B_w_up: jax.Array,
    B_w_down: jax.Array,
    c: jax.Array,
    w_mod: jax.Array,
):
    del B_x
    B, S, M = A_x.shape
    Dc = A_c_kv.shape[2]
    _, H, D = A_w_q.shape
    F = B_w_down.shape[0]
    assert B == 1 and A_c_kv.shape[1] == S
    assert S == sum(_CKV_ROWS) == sum(_PROJ_ROWS) == sum(_OUT_ROWS)

    args = (
        A_x.reshape(S, M), A_c_kv.reshape(S, Dc), A_w_q, A_w_uk, A_w_uv,
        A_w_o.reshape(H * D, M), w_mod, B_w_gate.T, B_w_up.T, B_w_down, B_w_r, c,
    )
    ng = H // _HG
    scratch = [
        pltpu.VMEM((H, S // 2, D), U32),
        pltpu.VMEM((H, S // 2, D), U32),
        pltpu.VMEM((H, S // 2, D), U32),
        pltpu.VMEM((S // 2, M), U32),
        pltpu.VMEM((H // 2, M // 2, 2 * D), U32),
        pltpu.VMEM((_HG, Dc // 2, 2 * D), U32),
        pltpu.VMEM((S, M), F32),
        pltpu.VMEM((S, M), F32),
        pltpu.VMEM((S, M), BF16),
        pltpu.VMEM((_RGR * _HG // 2, D), U32),
        pltpu.VMEM((M, 128), F32),
        pltpu.VMEM((2, M // 2, F), U32),
    ] + [
        pltpu.VMEM((ng, a.shape[0], _HG, D) if a.ndim == 3 else a.shape, a.dtype)
        for a in args
    ] + [
        pltpu.VMEM((8, M), F32),
        pltpu.SemaphoreType.DMA((3 * ng + len(_CKV_ROWS) + 9,)),
        pltpu.SemaphoreType.DMA((len(_OUT_ROWS),)),
        pltpu.SemaphoreType.DMA((_TOPC,)),
    ]

    out = pl.pallas_call(
        _kernel,
        in_specs=[pl.BlockSpec(memory_space=pltpu.HBM)] * len(args),
        out_specs=pl.BlockSpec(memory_space=pltpu.HBM),
        out_shape=jax.ShapeDtypeStruct((S, M), A_x.dtype),
        scratch_shapes=scratch,
        compiler_params=pltpu.CompilerParams(vmem_limit_bytes=120 * 1024 * 1024),
        name="adaln_cla_mod",
    )(*args)
    return out.reshape(B, S, M)
```
